```python
import os as _os
_os.environ.setdefault('JAX_PLATFORMS', 'cpu')
import jax
import jax.numpy as jnp

def _softmax(x, axis=-1):
    return jax.nn.softmax(x, axis=axis)

def _gelu(x):
    return jax.nn.gelu(x, approximate=True)

def _silu(x):
    return jax.nn.silu(x)

def _sigmoid(x):
    return jax.nn.sigmoid(x)

def _layernorm(x, axis=-1, eps=1e-05):
    m = jnp.mean(x, axis=axis, keepdims=True)
    v = jnp.var(x, axis=axis, keepdims=True)
    return (x - m) / jnp.sqrt(v + eps)

def _scatter_add(tgt, idx, src, axis=0):
    return tgt.at[idx].add(src)

def _segment_sum(src, seg, n):
    return jax.ops.segment_sum(src, seg, n)

class _Rng:

    def __init__(self, key):
        self._k = key

    def _next(self):
        self._k, sub = jax.random.split(self._k)
        return sub

    def normal(self, shape):
        return jax.random.normal(self._next(), shape, dtype=jnp.bfloat16)

    def randint(self, lo, hi, shape):
        return jax.random.randint(self._next(), shape, lo, hi, dtype=jnp.int32)

    def uniform(self, shape, lo=0.0, hi=1.0):
        return jax.random.uniform(self._next(), shape, jnp.bfloat16, lo, hi)

    def permutation(self, n):
        return jax.random.permutation(self._next(), n)
kernel_name = 'adaLN_cond__sliding_local_dilated__dense_activation_silu__prompt'

def setup_inputs():
    _rng = _Rng(jax.random.key(int.from_bytes(__import__("os").urandom(4), "little")))
    _w = lambda a: (lambda t: t.astype(jnp.bfloat16) if jnp.issubdtype(t.dtype, jnp.floating) else t)(jnp.asarray(a))

    def _A_setup():
        B, S, D = (1, 2048, 512)
        return {'x': _w((lambda *s: _rng.normal(s) * 0.05)(B, S, D)), 'wqkv': _w((lambda *s: _rng.normal(s) * 0.05)(D, 3 * D)), 'wo': _w((lambda *s: _rng.normal(s) * 0.05)(D, D))}
    _A_in = _A_setup()

    def _B_setup():
        B, S, D, F = (1, 2048, 512, 1792)
        return {'x': _w((lambda *s: _rng.normal(s) * 0.05)(B, S, D)), 'w1': _w((lambda *s: _rng.normal(s) * 0.8)(D, F) * D ** (-0.5)), 'w2': _w((lambda *s: _rng.normal(s) * 0.8)(F, D) * F ** (-0.5))}
    _B_in = _B_setup()
    return {'A_x': _A_in['x'], 'A_wqkv': _A_in['wqkv'], 'A_wo': _A_in['wo'], 'B_x': _B_in['x'], 'B_w1': _B_in['w1'], 'B_w2': _B_in['w2'], 'c': _w((lambda *s: _rng.normal(s) * 0.05)(1, 512) * 8.0), 'w_mod': _w((lambda *s: _rng.normal(s) * 0.05)(512, 6 * 512) * 512 ** (-0.5) * 8.0)}

def reference(A_x, A_wqkv, A_wo, B_x, B_w1, B_w2, c, w_mod):

    def _A_ref(x, wqkv, wo):
        B, S, D = x.shape
        H = 32
        Dh = D // H
        W, dil = (8, 2)
        qkv = (lambda x, *d: x.transpose(*d))((x @ wqkv).reshape(B, S, 3, H, Dh), 2, 0, 3, 1, 4)
        q, k, v = (qkv[0], qkv[1], qkv[2])
        scale = Dh ** (-0.5)
        pos = jnp.arange(S)
        off = jnp.arange(W) * dil
        idx = pos[:, None] - off[None, :]
        mask = idx >= 0
        idx_c = jnp.where(mask, idx, 0).reshape(-1)
        kg = k[:, :, idx_c, :].reshape(B, H, S, W, Dh)
        vg = v[:, :, idx_c, :].reshape(B, H, S, W, Dh)
        logits = jnp.einsum('bhsd,bhswd->bhsw', q, kg) * scale
        logits = jnp.where(mask[None, None, :, :], logits, -1000000000.0)
        attn = _softmax(logits, axis=-1)
        o = jnp.einsum('bhsw,bhswd->bhsd', attn, vg)
        return (lambda x, *d: x.transpose(*d))(o, 0, 2, 1, 3).reshape(B, S, D) @ wo

    def _B_ref(x, w1, w2):
        h = jnp.einsum('bsd,df->bsf', x, w1)
        h = _silu(h)
        out = jnp.einsum('bsf,fd->bsd', h, w2)
        return out
    x = A_x
    mod = (_silu(c) @ w_mod).reshape(c.shape[0], 6, 1, -1)
    sa, ca, ga, sb, cb, gb = (mod[:, 0].copy(), mod[:, 1].copy(), mod[:, 2].copy(), mod[:, 3].copy(), mod[:, 4].copy(), mod[:, 5].copy())
    h = _layernorm(x, axis=-1) * (1 + ca) + sa
    x = x + ga * _A_ref(h, A_wqkv, A_wo)
    h = _layernorm(x, axis=-1) * (1 + cb) + sb
    x = x + gb * _B_ref(h, B_w1, B_w2)
    return x
```

```python
import functools
import jax
import jax.numpy as jnp
from jax import lax
import jax.experimental.pallas as pl
import jax.experimental.pallas.tpu as pltpu

F32 = jnp.float32
BF16 = jnp.bfloat16
U32 = jnp.uint32
H = 32
DH = 16
W = 8
DIL = 2
HALO = 16
T = 256
R = 8
D = 512
NC = D // 128
FC = 256
LR = 32


def _ln(x):
    m = jnp.mean(x, axis=-1, keepdims=True)
    xc = x - m
    v = jnp.mean(xc * xc, axis=-1, keepdims=True)
    return xc * lax.rsqrt(v + 1e-5)


def _silu(u):
    return u * (0.5 * jnp.tanh(0.5 * u) + 0.5)


def _zero_of(tok):
    z = pltpu.bitcast(tok, U32)
    return lax.shift_right_logical(lax.shift_right_logical(z, U32(16)), U32(16))


def _gate(v, z):
    reps = (v.shape[0] // 8, v.shape[1] // 128)
    zz = z if reps == (1, 1) else jnp.tile(z, reps)
    return pltpu.bitcast(pltpu.bitcast(v, U32) | zz, F32)


def _kernel(x_ref, xp_ref, wqkv_ref, wo_ref, w1_ref, w2_ref, c_ref, wmod_ref, o_ref,
            wqkv_p, wo_p, mod_ref, q_s, k_s, v_s, a_s, *, n_tiles):
    i = pl.program_id(0)
    Fd = w1_ref.shape[1]

    def mod(k):
        return mod_ref[0:1, k * D:(k + 1) * D]

    def prologue():
        c = c_ref[...].astype(F32)
        sc = (c * jax.nn.sigmoid(c)).astype(BF16)
        sc8 = jnp.broadcast_to(sc, (8, D))
        mod_ref[...] = jnp.dot(sc8, wmod_ref[...], preferred_element_type=F32)
        src = lax.broadcasted_iota(jnp.int32, (D, D), 0)
        dst = lax.broadcasted_iota(jnp.int32, (D, D), 1)
        P = jnp.where(src == (dst % H) * DH + dst // H, 1.0, 0.0).astype(BF16)
        PT = jnp.where(dst == (src % H) * DH + src // H, 1.0, 0.0).astype(BF16)
        for j in range(3):
            wqkv_p[:, j * D:(j + 1) * D] = jnp.dot(
                wqkv_ref[:, j * D:(j + 1) * D], P, preferred_element_type=F32).astype(BF16)
        wo_p[...] = jnp.dot(PT, wo_ref[...], preferred_element_type=F32).astype(BF16)
        k_s[:, 0:HALO, :] = jnp.zeros((NC, HALO, 128), F32)
        v_s[:, 0:HALO, :] = jnp.zeros((NC, HALO, 128), F32)

    def a_qkv(first):
        if not first:
            k_s[:, 0:HALO, :] = k_s[:, T:T + HALO, :]
            v_s[:, 0:HALO, :] = v_s[:, T:T + HALO, :]
        x = x_ref[...].astype(F32)
        h = (_ln(x) * (1.0 + mod(1)) + mod(0)).astype(BF16)
        qkv = jnp.dot(h, wqkv_p[...], preferred_element_type=F32)
        scale = DH ** -0.5
        for j in range(NC):
            q_s[j] = qkv[:, j * 128:(j + 1) * 128] * scale
            k_s[j, HALO:HALO + T, :] = qkv[:, D + j * 128:D + (j + 1) * 128]
            v_s[j, HALO:HALO + T, :] = qkv[:, 2 * D + j * 128:2 * D + (j + 1) * 128]

    def a_attn(first, tokens=None):
        n = T // R
        for r in range(n):
            r0 = r * R
            q = [q_s[j, r0:r0 + R, :] for j in range(NC)]
            if tokens is not None:
                z = _zero_of(tokens[r * (len(tokens) - 6) // n])
                q = [_gate(qq, z) for qq in q]
            logits = []
            for w in range(W):
                s0 = HALO + r0 - DIL * w
                t = q[0] * k_s[0, s0:s0 + R, :]
                for j in range(1, NC):
                    t = t + q[j] * k_s[j, s0:s0 + R, :]
                t = t + pltpu.roll(t, 64, 1)
                t = t + pltpu.roll(t, 32, 1)
                if first and r0 < HALO and w > 0:
                    row = r0 + lax.broadcasted_iota(jnp.int32, (R, 128), 0)
                    t = jnp.where(row >= DIL * w, t, -1e9)
                logits.append(t)
            m = logits[0]
            for w in range(1, W):
                m = jnp.maximum(m, logits[w])
            ps = [jnp.exp(l - m) for l in logits]
            den = ps[0]
            for w in range(1, W):
                den = den + ps[w]
            inv = 1.0 / den
            for j in range(NC):
                acc = None
                for w in range(W):
                    s0 = HALO + r0 - DIL * w
                    term = ps[w] * v_s[j, s0:s0 + R, :]
                    acc = term if acc is None else acc + term
                a_s[r0:r0 + R, j * 128:(j + 1) * 128] = (acc * inv).astype(BF16)

    def b_wo():
        att = jnp.dot(a_s[...], wo_p[...], preferred_element_type=F32)
        return xp_ref[...].astype(F32) + mod(2) * att

    def b_ffn(x1):
        h2 = (_ln(x1) * (1.0 + mod(4)) + mod(3)).astype(BF16)
        nch = Fd // FC
        toks = []
        us = []
        y = None

        def w1c(c):
            u = jnp.dot(h2, w1_ref[:, c * FC:(c + 1) * FC], preferred_element_type=F32)
            for cb in range(FC // 128):
                for row in (0, T // 2):
                    toks.append(u[row:row + 8, cb * 128:(cb + 1) * 128])
            us.append(_silu(u).astype(BF16))

        def w2c(c, y):
            p = jnp.dot(us[c], w2_ref[c * FC:(c + 1) * FC, :], preferred_element_type=F32)
            for cb in (0, 2):
                for row in (0, T // 2):
                    toks.append(p[row:row + 8, cb * 128:(cb + 1) * 128])
            return p if y is None else y + p

        w1c(0)
        for c in range(nch):
            if c + 1 < nch:
                w1c(c + 1)
            y = w2c(c, y)
        o_ref[...] = (x1 + mod(5) * y).astype(o_ref.dtype)
        return toks

    @pl.when(i == 0)
    def _():
        prologue()
        a_qkv(True)
        a_attn(True)

    @pl.when(jnp.logical_and(i > 0, i < n_tiles))
    def _():
        x1 = b_wo()
        a_qkv(False)
        toks = b_ffn(x1)
        a_attn(False, toks)

    @pl.when(i == n_tiles)
    def _():
        x1 = b_wo()
        b_ffn(x1)


@jax.jit
def pallas_adaLN_cond__sliding_local_dilated__dense_activation_silu__prompt_kernel(
    A_x, A_wqkv, A_wo, B_x, B_w1, B_w2, c, w_mod,
):
    B, S, _ = A_x.shape
    Fd = B_w1.shape[1]
    n = S // T
    x2 = A_x.reshape(S, D)
    full = lambda shape: pl.BlockSpec(shape, lambda i: (0,) * len(shape))
    out = pl.pallas_call(
        functools.partial(_kernel, n_tiles=n),
        grid=(n + 1,),
        in_specs=[
            pl.BlockSpec((T, D), lambda i: (jnp.minimum(i, n - 1), 0)),
            pl.BlockSpec((T, D), lambda i: (jnp.maximum(i - 1, 0), 0)),
            full((D, 3 * D)), full((D, D)), full((D, Fd)), full((Fd, D)),
            full((1, D)), full((D, 6 * D)),
        ],
        out_specs=pl.BlockSpec((T, D), lambda i: (jnp.maximum(i - 1, 0), 0)),
        out_shape=jax.ShapeDtypeStruct((S, D), A_x.dtype),
        scratch_shapes=[
            pltpu.VMEM((D, 3 * D), BF16),
            pltpu.VMEM((D, D), BF16),
            pltpu.VMEM((8, 6 * D), F32),
            pltpu.VMEM((NC, T, 128), F32),
            pltpu.VMEM((NC, T + HALO, 128), F32),
            pltpu.VMEM((NC, T + HALO, 128), F32),
            pltpu.VMEM((T, D), BF16),
        ],
        compiler_params=pltpu.CompilerParams(
            dimension_semantics=("arbitrary",),
            vmem_limit_bytes=64 * 1024 * 1024,
        ),
    )(x2, x2, A_wqkv, A_wo, B_w1, B_w2, c, w_mod)
    return out.reshape(B, S, D)
```

```python
import functools
import jax
import jax.numpy as jnp
from jax import lax
import jax.experimental.pallas as pl
import jax.experimental.pallas.tpu as pltpu

F32 = jnp.float32
BF16 = jnp.bfloat16
U32 = jnp.uint32
I32 = jnp.int32
H = 32
DH = 16
W = 8
DIL = 2
HALO = 16
T = 256
R = 8
D = 512
KH = D // 2
NC = D // 128
FC = 256
LR = 16
NL = T // LR
NR = T // R
SLOTS = 3
TA = 6
LOG2E = 1.4426950408889634
QSCALE = DH ** -0.5 * LOG2E


def _ln(x):
    m = jnp.mean(x, axis=-1, keepdims=True)
    xc = x - m
    v = jnp.mean(xc * xc, axis=-1, keepdims=True)
    return xc * lax.rsqrt(v + 1e-5)


def _silu(u):
    return u * (0.5 * jnp.tanh(0.5 * u) + 0.5)


def _zero_of(tok):
    z = pltpu.bitcast(tok, U32)
    return lax.shift_right_logical(lax.shift_right_logical(z, U32(16)), U32(16))


def _gate(v, tok):
    if tok is None:
        return v
    z = _zero_of(tok)
    u = pltpu.bitcast(v, U32)
    reps = (u.shape[0] // 8, u.shape[1] // 128)
    zz = z if reps == (1, 1) else jnp.tile(z, reps)
    return pltpu.bitcast(u | zz, v.dtype)


def _spread(jobs, toks):
    extra = None
    for k, job in enumerate(jobs):
        tok = toks[k * len(toks) // len(jobs)] if toks else None
        if extra is not None:
            tok = extra if tok is None else tok + extra
        extra = job(tok)


def _merge(a, b):
    out = []
    j = 0
    for i, x in enumerate(a):
        out.append(x)
        while j < len(b) and (j + 1) * len(a) <= (i + 1) * (len(b) + 1) and j < len(b):
            out.append(b[j])
            j += 1
    out.extend(b[j:])
    return out


def _kernel(x_hbm, wqkv_hbm, wo_hbm, w1_hbm, w2_hbm, c_hbm, wmod_hbm, o_hbm,
            x_v, o_v, wqkv_v, wo_v, w1_v, w2_v, c_v, wmod_v,
            wqkv_p, wo_p, mod_ref, q_s, k_s, v_s, a_s, h1_s, h2_s, x1_s,
            sem_in, sem_out, *, n, nch):
    cps = {}
    order = []

    def add(name, src, dst):
        cps[name] = pltpu.make_async_copy(src, dst, sem_in.at[len(order)])
        order.append(name)

    def xt(a, b):
        return x_hbm.at[pl.ds(a * T, (b - a) * T)], x_v.at[pl.ds(a * T, (b - a) * T)]

    def mcols(c0, nc):
        return wmod_hbm.at[:, pl.ds(c0, nc)], wmod_v.at[:, pl.ds(c0, nc)]

    add('c', c_hbm, c_v)
    add('x0', *xt(0, 1))
    add('W0', wqkv_hbm.at[pl.ds(0, KH)], wqkv_v.at[pl.ds(0, KH)])
    add('sa0', *mcols(0, KH))
    add('ca0', *mcols(D, KH))
    add('x1', *xt(1, 2))
    add('W1', wqkv_hbm.at[pl.ds(KH, KH)], wqkv_v.at[pl.ds(KH, KH)])
    add('sa1', *mcols(KH, KH))
    add('ca1', *mcols(D + KH, KH))
    add('x2', *xt(2, 3))
    add('wo', wo_hbm, wo_v)
    add('m1', *mcols(2 * D, 4 * D))
    for c in range(nch):
        add(f'w1_{c}', w1_hbm.at[:, pl.ds(c * FC, FC)], w1_v.at[c])
        add(f'w2_{c}', w2_hbm.at[pl.ds(c * FC, FC)], w2_v.at[c])
    add('xr', *xt(3, n))
    for name in order:
        cps[name].start()

    def wait(*names):
        for name in names:
            cps[name].wait()

    def mod(k, c0=0, c1=D):
        return mod_ref[0:1, k * D + c0:k * D + c1]

    def rows(t, r0=0, nr=T):
        if isinstance(t, int):
            return pl.ds(t * T + r0, nr)
        return pl.ds(pl.multiple_of(t * T + r0, nr), nr)

    def calc_mod(c0, c1):
        c = c_v[...].astype(F32)
        sc = (c * jax.nn.sigmoid(c)).astype(BF16)
        sc8 = jnp.broadcast_to(sc, (8, D))
        mod_ref[:, c0:c1] = jnp.dot(sc8, wmod_v[:, c0:c1], preferred_element_type=F32)

    def perm_mats():
        src = lax.broadcasted_iota(I32, (128, 128), 0)
        m = lax.broadcasted_iota(I32, (128, 128), 1)
        out = []
        for i in range(NC):
            j = ((m >> 3) + (4 - i)) & 3
            l = (m + 128 - 8 * j) & 127
            out.append(jnp.where(src == (m & 7) * 16 + 4 * j + (l >> 5), 1.0, 0.0).astype(BF16))
        return out

    def perm_w(hf, Ls):
        rs = slice(hf * KH, (hf + 1) * KH)
        g = (lax.broadcasted_iota(I32, (KH // 2, 128), 1) >> 3) & 3
        for a in range(3):
            wp = [pltpu.bitcast(
                jnp.dot(wqkv_v[rs, a * D + i * 128:a * D + (i + 1) * 128], Ls[i],
                        preferred_element_type=F32).astype(BF16), U32) for i in range(NC)]
            for j in range(NC):
                pre = wp[(3 - j) % 4]
                for gg in (2, 1, 0):
                    pre = jnp.where(g == gg, wp[(gg - j) % 4], pre)
                if j:
                    pre = pltpu.roll(pre, 128 - 8 * j, 1)
                wqkv_p[rs, a * D + j * 128:a * D + (j + 1) * 128] = pltpu.bitcast(pre, BF16)

    def perm_wo():
        m = lax.broadcasted_iota(I32, (128, 128), 0)
        src = lax.broadcasted_iota(I32, (128, 128), 1)
        Lr = jnp.where(src == (m & 7) * 16 + (m >> 3), 1.0, 0.0).astype(BF16)
        rs = [jnp.dot(Lr, wo_v[i * 128:(i + 1) * 128, :], preferred_element_type=F32) for i in range(NC)]
        for d in range(DH):
            blk = jnp.concatenate([rs[i][8 * d:8 * d + 8, :] for i in range(NC)], axis=0)
            wo_p[d * H:(d + 1) * H, :] = blk.astype(BF16)

    def ln1_jobs(t, hs, chain=False):
        def job(r, tok):
            x = _gate(x_v[rows(t, r * LR, LR), :], tok).astype(F32)
            h = _ln(x) * (1.0 + mod(1)) + mod(0)
            h1_s[hs, r * LR:(r + 1) * LR, :] = h.astype(BF16)
            if chain:
                return h[0:8, 0:128] + h[8:16, 0:128]
        return [functools.partial(job, r) for r in range(NL)]

    def ln2_jobs(xs, r0=0, r1=NL):
        def job(r, tok):
            x1 = _gate(x1_s[xs, r * LR:(r + 1) * LR, :], tok)
            h2_s[r * LR:(r + 1) * LR, :] = (_ln(x1) * (1.0 + mod(4)) + mod(3)).astype(BF16)
        return [functools.partial(job, r) for r in range(r0, r1)]

    def tok_of(v, toks, cbs):
        for cb in cbs:
            for row in (0, v.shape[0] // 2):
                toks.append(v[row:row + 8, cb * 128:(cb + 1) * 128])

    def qkv_part(a, hs, sl, prev, toks, hf=None, chain=None):
        dst = (q_s, k_s, v_s)[a]
        if a and prev is not None:
            dst[sl, :, 0:HALO, :] = dst[prev, :, T:T + HALO, :]
        ks = slice(0, D) if hf is None else slice(hf * KH, (hf + 1) * KH)
        if chain is None:
            r = jnp.dot(h1_s[hs, :, ks], wqkv_p[ks, a * D:(a + 1) * D], preferred_element_type=F32)
        else:
            nw = 128 if hf is None else 256
            lhs = h1_s[hs, :, ks]
            parts = []
            for c0 in range(0, D, nw):
                w = wqkv_p[ks, a * D + c0:a * D + c0 + nw]
                if len(chain) >= LAG:
                    tk = chain[-LAG]
                    pcs = []
                    for k0 in range(0, w.shape[0], 128):
                        pcs += [_gate(w[k0:k0 + 16], tk), w[k0 + 16:k0 + 128]]
                    w = jnp.concatenate(pcs, axis=0)
                p = jnp.dot(lhs, w, preferred_element_type=F32)
                tk = p[T - 8:T, 0:128]
                if nw > 128:
                    tk = tk + p[T - 8:T, 128:256]
                chain.append(tk)
                parts.append(p)
            r = jnp.concatenate(parts, axis=1)
        tok_of(r, toks, range(NC))
        o = 0 if a == 0 else HALO
        for j in range(NC):
            rj = r[:, j * 128:(j + 1) * 128]
            if hf == 1:
                rj = rj + dst[sl, j, o:o + T, :]
            if a == 0 and hf != 0:
                rj = rj * QSCALE
            dst[sl, j, o:o + T, :] = rj

    def attn_jobs(sl, ra, rb, first=False):
        def job(r, tok):
            r0 = r * R
            q = [_gate(q_s[sl, j, r0:r0 + R, :], tok) for j in range(NC)]
            logits = []
            for w in range(W):
                s0 = HALO + r0 - DIL * w
                tt = q[0] * k_s[sl, 0, s0:s0 + R, :]
                for j in range(1, NC):
                    tt = tt + q[j] * k_s[sl, j, s0:s0 + R, :]
                tt = tt + pltpu.roll(tt, 64, 1)
                tt = tt + pltpu.roll(tt, 32, 1)
                if first and r0 < HALO and w > 0:
                    row = r0 + lax.broadcasted_iota(I32, (R, 128), 0)
                    tt = jnp.where(row >= DIL * w, tt, -1e9 * LOG2E)
                logits.append(tt)
            m = logits[0]
            for w in range(1, W):
                m = jnp.maximum(m, logits[w])
            ps = [jnp.exp2(l - m) for l in logits]
            den = ps[0]
            for w in range(1, W):
                den = den + ps[w]
            inv = 1.0 / den
            for j in range(NC):
                acc = None
                for w in range(W):
                    s0 = HALO + r0 - DIL * w
                    term = ps[w] * v_s[sl, j, s0:s0 + R, :]
                    acc = term if acc is None else acc + term
                a_s[r0:r0 + R, j * 128:(j + 1) * 128] = (acc * inv).astype(BF16)
        return [functools.partial(job, r) for r in range(ra, rb)]

    def wo_mm(t, xs, toks, r0=0, nr=T, ln=False):
        att = jnp.dot(a_s[r0:r0 + nr, :], wo_p[...], preferred_element_type=F32)
        tok_of(att, toks, range(NC))
        x1 = x_v[rows(t, r0, nr), :].astype(F32) + mod(2) * att
        x1_s[xs, r0:r0 + nr, :] = x1
        if ln:
            h2_s[r0:r0 + nr, :] = (_ln(x1) * (1.0 + mod(4)) + mod(3)).astype(BF16)

    def out_copy(t):
        return pltpu.make_async_copy(o_v.at[rows(t)], o_hbm.at[rows(t)], sem_out.at[t])

    def out_copy_col(t, j):
        cs = pl.ds(j * 128, 128)
        return pltpu.make_async_copy(o_v.at[rows(t), cs], o_hbm.at[rows(t), cs], sem_out.at[t + j])

    class FFN:
        def __init__(self):
            self.us = []
            self.y = None

        def w1(self, c, toks, split=False):
            if split:
                u = jnp.concatenate([
                    jnp.dot(h2_s[hh * (T // 2):(hh + 1) * (T // 2), :], w1_v[c], preferred_element_type=F32)
                    for hh in range(2)], axis=0)
            else:
                u = jnp.dot(h2_s[...], w1_v[c], preferred_element_type=F32)
            tok_of(u, toks, range(FC // 128))
            self.us.append(_silu(u).astype(BF16))

        def w2(self, c, toks):
            p = jnp.dot(self.us[c], w2_v[c], preferred_element_type=F32)
            tok_of(p, toks, (0, 2))
            self.y = p if self.y is None else self.y + p

        def run(self, seq, toks):
            for kind, c in seq:
                (self.w1 if kind == 1 else self.w2)(c, toks)

        def fin(self, t, xs):
            o_v[rows(t), :] = (x1_s[xs] + mod(5) * self.y).astype(BF16)

        def fin_cols(self, t, xs):
            uu = jnp.concatenate(self.us[nch - 2:], axis=1)
            for j in range(NC):
                cs = slice(j * 128, (j + 1) * 128)
                wj = jnp.concatenate([w2_v[nch - 2, :, cs], w2_v[nch - 1, :, cs]], axis=0)
                y = self.y[:, cs] + jnp.dot(uu, wj, preferred_element_type=F32)
                o_v[rows(t), cs] = (x1_s[xs, :, cs] + mod(5, j * 128, (j + 1) * 128) * y).astype(BF16)
                out_copy_col(t, j).start()

    SEQ = [(1, 0)]
    for c in range(nch):
        if c + 1 < nch:
            SEQ.append((1, c + 1))
        SEQ.append((2, c))

    def body(t, carry):
        f = FFN()
        toks = []
        f.run(SEQ, toks)
        _spread(_merge(attn_jobs(0, 0, NR), ln1_jobs(t + 2, 0, True)), toks[:len(toks) - TA])
        f.fin(t, 0)
        wo_mm(t + 1, 0, [], ln=True)
        for a in range(3):
            qkv_part(a, 0, 0, 0, [])
        out_copy(t).start()
        return carry

    def modulate(hs, hf):
        cs = slice(hf * KH, (hf + 1) * KH)
        h1_s[hs, :, cs] = (x1_s[hs, :, cs] * (1.0 + mod(1, hf * KH, (hf + 1) * KH))
                           + mod(0, hf * KH, (hf + 1) * KH)).astype(BF16)

    k_s[2, :, 0:HALO, :] = jnp.zeros((NC, HALO, 128), F32)
    v_s[2, :, 0:HALO, :] = jnp.zeros((NC, HALO, 128), F32)
    Ls = perm_mats()
    wait('c', 'x0')
    x1_s[0] = _ln(x_v[rows(0), :].astype(F32))
    wait('W0')
    perm_w(0, Ls)
    wait('sa0', 'ca0')
    calc_mod(0, KH)
    calc_mod(D, D + KH)
    modulate(0, 0)
    for a in range(3):
        qkv_part(a, 0, 2, None, [], 0)
    wait('x1', 'W1')
    perm_w(1, Ls)
    x1_s[1] = _ln(x_v[rows(1), :].astype(F32))
    modulate(1, 0)
    for a in range(3):
        qkv_part(a, 1, 1, None, [], 0)
    wait('sa1', 'ca1', 'x2', 'wo')
    calc_mod(KH, D)
    calc_mod(D + KH, 2 * D)
    perm_wo()
    modulate(0, 1)
    modulate(1, 1)
    tk0 = []
    ch = []
    for a in range(3):
        qkv_part(a, 0, 2, None, tk0, 1, ch)
    _spread(ln1_jobs(2, 2), tk0[:20])
    toks = []
    for a in range(3):
        qkv_part(a, 1, 1, 2, toks, 1, ch)
    toks = toks[::2]
    for a in range(3):
        qkv_part(a, 2, 0, 1, toks, None, ch)
    _spread(attn_jobs(2, 0, NR, first=True), [None] + toks[:-2])
    wait('m1', *[f'w{k}_{c}' for c in range(P0) for k in (1, 2)])
    calc_mod(2 * D, 5 * D)
    toks = []
    wo_mm(0, 1, toks, 0, T // 2, ln=True)
    wo_mm(0, 1, toks, T // 2, T // 2, ln=True)
    calc_mod(5 * D, 6 * D)
    f = FFN()
    toks = []
    seq0 = [s for s in SEQ if s[1] < P0]
    seq1 = [s for s in SEQ if s not in seq0]
    f.w1(0, toks, split=True)
    f.run(seq0[1:], toks)
    _spread(attn_jobs(1, 0, A1), toks[:-3])
    wait(*[f'w{k}_{c}' for c in range(P0, nch) for k in (1, 2)])
    toks = []
    f.run(seq1[:-2], toks)
    _spread(attn_jobs(1, A1, NR), [None] + toks[:-4])
    wo_mm(1, 0, [], ln=True)
    f.run(seq1[-2:], [])
    f.fin(0, 1)
    out_copy(0).start()
    wait('xr')
    lax.fori_loop(1, n - 2 - PEEL, body, 0)
    for t in range(n - 2 - PEEL, n - 2):
        body(t, 0)
    f = FFN()
    toks = []
    f.run(SEQ[:-2], toks)
    _spread(attn_jobs(0, 0, NR), toks[:-6])
    wo_mm(n - 1, 1, [], ln=True)
    f.run(SEQ[-2:], [])
    f.fin(n - 2, 0)
    f = FFN()
    f.run(SEQ[:3], [])
    out_copy(n - 2).start()
    f.run(SEQ[3:-2], [])
    f.fin_cols(n - 1, 1)
    for t in range(n - 1):
        out_copy(t).wait()
    for j in range(NC):
        out_copy_col(n - 1, j).wait()


A1 = 15
P0 = 3
PEEL = 0
LAG = 3


@jax.jit
def pallas_adaLN_cond__sliding_local_dilated__dense_activation_silu__prompt_kernel(
    A_x, A_wqkv, A_wo, B_x, B_w1, B_w2, c, w_mod,
):
    B, S, _ = A_x.shape
    Fd = B_w1.shape[1]
    n = S // T
    nch = Fd // FC
    x2 = A_x.reshape(S, D)
    anyspec = pl.BlockSpec(memory_space=pl.ANY)
    out = pl.pallas_call(
        functools.partial(_kernel, n=n, nch=nch),
        in_specs=[anyspec] * 7,
        out_specs=anyspec,
        out_shape=jax.ShapeDtypeStruct((S, D), A_x.dtype),
        scratch_shapes=[
            pltpu.VMEM((S, D), BF16),
            pltpu.VMEM((S, D), BF16),
            pltpu.VMEM((D, 3 * D), BF16),
            pltpu.VMEM((D, D), BF16),
            pltpu.VMEM((nch, D, FC), BF16),
            pltpu.VMEM((nch, FC, D), BF16),
            pltpu.VMEM((1, D), BF16),
            pltpu.VMEM((D, 6 * D), BF16),
            pltpu.VMEM((D, 3 * D), BF16),
            pltpu.VMEM((D, D), BF16),
            pltpu.VMEM((8, 6 * D), F32),
            pltpu.VMEM((SLOTS, NC, T, 128), F32),
            pltpu.VMEM((SLOTS, NC, T + HALO, 128), F32),
            pltpu.VMEM((SLOTS, NC, T + HALO, 128), F32),
            pltpu.VMEM((T, D), BF16),
            pltpu.VMEM((3, T, D), BF16),
            pltpu.VMEM((T, D), BF16),
            pltpu.VMEM((2, T, D), F32),
            pltpu.SemaphoreType.DMA((13 + 2 * nch,)),
            pltpu.SemaphoreType.DMA((n + NC - 1,)),
        ],
        compiler_params=pltpu.CompilerParams(vmem_limit_bytes=100 * 1024 * 1024),
    )(x2, A_wqkv, A_wo, B_w1, B_w2, c, w_mod)
    return out.reshape(B, S, D)
```

```python
import functools
import jax
import jax.numpy as jnp
from jax import lax
import jax.experimental.pallas as pl
import jax.experimental.pallas.tpu as pltpu

F32 = jnp.float32
BF16 = jnp.bfloat16
U32 = jnp.uint32
I32 = jnp.int32
H = 32
DH = 16
W = 8
DIL = 2
HALO = 16
T = 256
R = 8
D = 512
KH = D // 2
NC = D // 128
FC = 256
LR = 16
NL = T // LR
NR = T // R
SLOTS = 4
TA = 6
LOG2E = 1.4426950408889634
QSCALE = DH ** -0.5 * LOG2E


def _ln(x):
    m = jnp.mean(x, axis=-1, keepdims=True)
    xc = x - m
    v = jnp.mean(xc * xc, axis=-1, keepdims=True)
    return xc * lax.rsqrt(v + 1e-5)


def _silu(u):
    return u * (0.5 * jnp.tanh(0.5 * u) + 0.5)


def _zero_of(tok):
    z = pltpu.bitcast(tok, U32)
    return lax.shift_right_logical(lax.shift_right_logical(z, U32(16)), U32(16))


def _gate(v, tok):
    if tok is None:
        return v
    z = _zero_of(tok)
    u = pltpu.bitcast(v, U32)
    reps = (u.shape[0] // 8, u.shape[1] // 128)
    zz = z if reps == (1, 1) else jnp.tile(z, reps)
    return pltpu.bitcast(u | zz, v.dtype)


def _spread(jobs, toks):
    extra = None
    for k, job in enumerate(jobs):
        tok = toks[k * len(toks) // len(jobs)] if toks else None
        if extra is not None:
            tok = extra if tok is None else tok + extra
        extra = job(tok)
    return extra


def _par(jobs, toks):
    out = None
    for k, job in enumerate(jobs):
        r = job(toks[k * len(toks) // len(jobs)] if toks else None)
        out = r if out is None else out + r
    return out


def _merge(a, b):
    out = []
    j = 0
    for i, x in enumerate(a):
        out.append(x)
        while j < len(b) and (j + 1) * len(a) <= (i + 1) * (len(b) + 1) and j < len(b):
            out.append(b[j])
            j += 1
    out.extend(b[j:])
    return out


def _kernel(x_hbm, wqkv_hbm, wo_hbm, w1_hbm, w2_hbm, c_hbm, wmod_hbm, o_hbm,
            x_v, o_v, wqkv_v, wo_v, w1_v, w2_v, c_v, wmod_v,
            wqkv_p, wo_p, mod_ref, sct, q_s, k_s, v_s, a_s, h1_s, h2_s, x1_s,
            sem_in, sem_out, *, n, nch):
    cps = {}
    order = []

    def add(name, src, dst):
        cps[name] = pltpu.make_async_copy(src, dst, sem_in.at[len(order)])
        order.append(name)

    def xt(a, b):
        return x_hbm.at[pl.ds(a * T, (b - a) * T)], x_v.at[pl.ds(a * T, (b - a) * T)]

    def mcols(c0, nc):
        return wmod_hbm.at[:, pl.ds(c0, nc)], wmod_v.at[:, pl.ds(c0, nc)]

    add('c', c_hbm, c_v)
    add('x0', *xt(0, 1))

    def piece(i):
        k0, k1 = KP[i]
        add(f'sa{i}', *mcols(k0, k1 - k0))
        add(f'ca{i}', *mcols(D + k0, k1 - k0))
        add(f'W{i}', wqkv_hbm.at[pl.ds(k0, k1 - k0)], wqkv_v.at[pl.ds(k0, k1 - k0)])

    piece(0)
    add('x12', *xt(1, 3))
    piece(1)
    add('x3', *xt(3, 4))
    piece(2)
    add('wo', wo_hbm, wo_v)
    add('m1', *mcols(2 * D, 3 * D))
    for c in range(nch):
        if c == P0:
            add('gb', *mcols(5 * D, D))
        add(f'w1_{c}', w1_hbm.at[:, pl.ds(c * FC, FC)], w1_v.at[c])
        add(f'w2_{c}', w2_hbm.at[pl.ds(c * FC, FC)], w2_v.at[c])
    add('xr', *xt(4, n))
    for name in order:
        cps[name].start()

    def wait(*names):
        for name in names:
            cps[name].wait()

    def mod(k, c0=0, c1=D):
        return mod_ref[0:1, k * D + c0:k * D + c1]

    def rows(t, r0=0, nr=T):
        if isinstance(t, int):
            return pl.ds(t * T + r0, nr)
        return pl.ds(pl.multiple_of(t * T + r0, nr), nr)

    def make_sct():
        c = c_v[...].astype(F32)
        sc = (c * jax.nn.sigmoid(c)).astype(BF16).astype(F32)
        r = lax.broadcasted_iota(I32, (128, 128), 0)
        l = lax.broadcasted_iota(I32, (128, 128), 1)
        ones = jnp.ones((128, 128), BF16)
        for b in range(NC):
            dg = jnp.where(r == l, sc[:, b * 128:(b + 1) * 128], 0.0).astype(BF16)
            sct[b * 128:(b + 1) * 128, :] = jnp.dot(dg, ones, preferred_element_type=F32)

    def calc_mod(*rngs, nch=2, last=None):
        blocks = [c for c0, c1 in rngs for c in range(c0, c1, 128)]
        last = [None] * nch if last is None else list(last)
        for b0 in range(0, len(blocks), nch):
            grp = blocks[b0:b0 + nch]
            acc = [None] * len(grp)
            for g in range(D // 16):
                s = sct[g * 16:(g + 1) * 16, :]
                for bi, c in enumerate(grp):
                    p = wmod_v[g * 16:(g + 1) * 16, c:c + 128].astype(F32) * s
                    a = _gate(p[0:8], last[bi]) if acc[bi] is None else acc[bi] + p[0:8]
                    acc[bi] = a + p[8:16]
            for bi, c in enumerate(grp):
                mod_ref[0:1, c:c + 128] = jnp.sum(acc[bi], axis=0, keepdims=True)
                last[bi] = acc[bi]
        return last

    def tsum(ts):
        return functools.reduce(lambda u, v: u + v, ts)

    def perm_mats():
        src = lax.broadcasted_iota(I32, (128, 128), 0)
        m = lax.broadcasted_iota(I32, (128, 128), 1)
        out = []
        for i in range(NC):
            j = ((m >> 3) + (4 - i)) & 3
            l = (m + 128 - 8 * j) & 127
            out.append(jnp.where(src == (m & 7) * 16 + 4 * j + (l >> 5), 1.0, 0.0).astype(BF16))
        return out

    def perm_w(kr, Ls):
        rs = slice(kr[0], kr[1])
        ru = slice(kr[0] // 2, kr[1] // 2)
        m = lax.broadcasted_iota(I32, ((kr[1] - kr[0]) // 2, 128), 1)
        g = (m >> 3) & 3
        for a in range(3):
            wp = []
            for i in range(NC):
                w = wqkv_v[rs, a * D + i * 128:a * D + (i + 1) * 128]
                if Ls is None:
                    j = ((m >> 3) + (4 - i)) & 3
                    l = (m + 128 - 8 * j) & 127
                    idx = (m & 7) * 16 + 4 * j + (l >> 5)
                    wp.append(jnp.take_along_axis(pltpu.bitcast(w, U32), idx, axis=1))
                else:
                    wp.append(pltpu.bitcast(
                        jnp.dot(w, Ls[i], preferred_element_type=F32).astype(BF16), U32))
            for j in range(NC):
                pre = wp[(3 - j) % 4]
                for gg in (2, 1, 0):
                    pre = jnp.where(g == gg, wp[(gg - j) % 4], pre)
                if j:
                    pre = pltpu.roll(pre, 128 - 8 * j, 1)
                wqkv_p[ru, a * D + j * 128:a * D + (j + 1) * 128] = pre

    def wq(ks, c0, c1):
        return pltpu.bitcast(wqkv_p[ks.start // 2:ks.stop // 2, c0:c1], BF16)

    def perm_wo(tok=None):
        m = lax.broadcasted_iota(I32, (128, 128), 0)
        src = lax.broadcasted_iota(I32, (128, 128), 1)
        Lr = _gate(jnp.where(src == (m & 7) * 16 + (m >> 3), 1.0, 0.0).astype(BF16), tok)
        rs = [jnp.dot(Lr, wo_v[i * 128:(i + 1) * 128, :], preferred_element_type=F32) for i in range(NC)]
        for d in range(DH):
            blk = jnp.concatenate([rs[i][8 * d:8 * d + 8, :] for i in range(NC)], axis=0)
            wo_p[d * H:(d + 1) * H, :] = blk.astype(BF16)

    def ln1_jobs(t, hs, chain=False):
        def job(r, tok):
            x = _gate(x_v[rows(t, r * LR, LR), :], tok).astype(F32)
            h = _ln(x) * (1.0 + mod(1)) + mod(0)
            h1_s[hs, r * LR:(r + 1) * LR, :] = h.astype(BF16)
            if chain:
                return h[0:8, 0:128] + h[8:16, 0:128]
        return [functools.partial(job, r) for r in range(NL)]

    def ln2_jobs(xs, r0=0, r1=NL):
        def job(r, tok):
            x1 = _gate(x1_s[xs, r * LR:(r + 1) * LR, :], tok)
            h2_s[r * LR:(r + 1) * LR, :] = (_ln(x1) * (1.0 + mod(4)) + mod(3)).astype(BF16)
        return [functools.partial(job, r) for r in range(r0, r1)]

    def tok_of(v, toks, cbs, nr=2):
        for cb in cbs:
            for row in range(0, v.shape[0], v.shape[0] // nr):
                toks.append(v[row:row + 8, cb * 128:(cb + 1) * 128])

    def gate_rows(w, tok):
        if tok is None:
            return w
        pcs = []
        for k0 in range(0, w.shape[0], 128):
            pcs += [_gate(w[k0:k0 + 16], tok), w[k0 + 16:k0 + 128]]
        return jnp.concatenate(pcs, axis=0)

    def qkv_part(a, hs, sl, prev, toks, kr=(0, D), tok=None, j0=0, j1=NC):
        dst = (q_s, k_s, v_s)[a]
        if a and prev is not None:
            dst[sl, j0:j1, 0:HALO, :] = dst[prev, j0:j1, T:T + HALO, :]
        ks = slice(*kr)
        r = jnp.dot(h1_s[hs, :, ks], gate_rows(wq(ks, a * D + j0 * 128, a * D + j1 * 128), tok),
                    preferred_element_type=F32)
        tok_of(r, toks, range(0, j1 - j0, D // (kr[1] - kr[0])), 4)
        o = 0 if a == 0 else HALO
        for j in range(j0, j1):
            rj = r[:, (j - j0) * 128:(j - j0 + 1) * 128]
            if kr[0]:
                rj = rj + dst[sl, j, o:o + T, :]
            if a == 0 and kr[1] == D:
                rj = rj * QSCALE
            dst[sl, j, o:o + T, :] = rj

    def attn_jobs(sl, ra, rb, first=False, asl=0, thin=0):
        last = [None] * max(thin, 1)

        def job(r, tok):
            r0 = r * R
            q = [_gate(q_s[sl, j, r0:r0 + R, :], tok) for j in range(NC)]
            logits = []
            for w in range(W):
                s0 = HALO + r0 - DIL * w
                tt = q[0] * k_s[sl, 0, s0:s0 + R, :]
                for j in range(1, NC):
                    tt = tt + q[j] * k_s[sl, j, s0:s0 + R, :]
                tt = tt + pltpu.roll(tt, 64, 1)
                tt = tt + pltpu.roll(tt, 32, 1)
                if first and r0 < HALO and w > 0:
                    row = r0 + lax.broadcasted_iota(I32, (R, 128), 0)
                    tt = jnp.where(row >= DIL * w, tt, -1e9 * LOG2E)
                logits.append(tt)
            m = logits[0]
            for w in range(1, W):
                m = jnp.maximum(m, logits[w])
            ps = [jnp.exp2(l - m) for l in logits]
            den = ps[0]
            for w in range(1, W):
                den = den + ps[w]
            inv = 1.0 / den
            for j in range(NC):
                acc = None
                for w in range(W):
                    s0 = HALO + r0 - DIL * w
                    term = ps[w] * v_s[sl, j, s0:s0 + R, :]
                    if acc is None:
                        acc = _gate(term, last[j % thin]) if thin else term
                    else:
                        acc = acc + term
                if thin:
                    last[j % thin] = acc
                a_s[asl, r0:r0 + R, j * 128:(j + 1) * 128] = (acc * inv).astype(BF16)
        return [functools.partial(job, r) for r in range(ra, rb)]

    def wo_mm(t, xs, toks, r0=0, nr=T, ln=False, asl=0, tok=None):
        att = jnp.dot(a_s[asl, r0:r0 + nr, :], gate_rows(wo_p[...], tok), preferred_element_type=F32)
        tok_of(att, toks, range(NC))
        x1 = x_v[rows(t, r0, nr), :].astype(F32) + mod(2) * att
        x1_s[xs, r0:r0 + nr, :] = x1
        if ln:
            h2_s[r0:r0 + nr, :] = (_ln(x1) * (1.0 + mod(4)) + mod(3)).astype(BF16)

    def out_copy(t):
        return pltpu.make_async_copy(o_v.at[rows(t)], o_hbm.at[rows(t)], sem_out.at[t])

    def out_copy_col(t, j):
        cs = pl.ds(j * 128, 128)
        return pltpu.make_async_copy(o_v.at[rows(t), cs], o_hbm.at[rows(t), cs], sem_out.at[t + j])

    class FFN:
        def __init__(self):
            self.us = []
            self.y = None

        def w1(self, c, toks, split=False):
            if split:
                u = jnp.concatenate([
                    jnp.dot(h2_s[hh * (T // 2):(hh + 1) * (T // 2), :], w1_v[c], preferred_element_type=F32)
                    for hh in range(2)], axis=0)
            else:
                u = jnp.dot(h2_s[...], w1_v[c], preferred_element_type=F32)
            tok_of(u, toks, range(FC // 128))
            self.us.append(_silu(u).astype(BF16))

        def w2(self, c, toks):
            p = jnp.dot(self.us[c], w2_v[c], preferred_element_type=F32)
            tok_of(p, toks, (0, 2))
            self.y = p if self.y is None else self.y + p

        def run(self, seq, toks):
            for kind, c in seq:
                (self.w1 if kind == 1 else self.w2)(c, toks)

        def fin(self, t, xs):
            o_v[rows(t), :] = (x1_s[xs] + mod(5) * self.y).astype(BF16)

        def fin_cols(self, t, xs):
            uu = jnp.concatenate(self.us[nch - 2:], axis=1)
            for j in range(NC):
                cs = slice(j * 128, (j + 1) * 128)
                wj = jnp.concatenate([w2_v[nch - 2, :, cs], w2_v[nch - 1, :, cs]], axis=0)
                y = self.y[:, cs] + jnp.dot(uu, wj, preferred_element_type=F32)
                o_v[rows(t), cs] = (x1_s[xs, :, cs] + mod(5, j * 128, (j + 1) * 128) * y).astype(BF16)
                out_copy_col(t, j).start()

    SEQ = [(1, 0)]
    for c in range(nch):
        if c + 1 < nch:
            SEQ.append((1, c + 1))
        SEQ.append((2, c))

    def body(t, carry):
        sl = (t + 1) & 1
        f = FFN()
        toks = []
        f.run(SEQ, toks)
        _spread(_merge(attn_jobs(sl, 0, NR, thin=TH2), ln1_jobs(t + 3, 0, True)), toks[:len(toks) - TA])
        f.fin(t, 0)
        wo_mm(t + 1, 0, [], ln=True)
        for a in range(3):
            qkv_part(a, 0, sl, 1 - sl, [])
        out_copy(t).start()
        return carry

    def fold(h):
        parts = [h[r:r + 8, c:c + 128] for r in range(0, h.shape[0], 8) for c in range(0, h.shape[1], 128)]
        return tsum(parts)

    def ln0_jobs(t, hs, k1):
        def job(r, tok):
            rs = slice(r * LR, (r + 1) * LR)
            y = _ln(_gate(x_v[rows(t, r * LR, LR), :], tok).astype(F32))
            x1_s[hs, rs, k1:] = y[:, k1:]
            h = y[:, :k1] * (1.0 + mod(1, 0, k1)) + mod(0, 0, k1)
            h1_s[hs, rs, :k1] = h.astype(BF16)
            return h[0:8, 0:128] + h[8:16, 0:128] + y[0:8, 256:384] + y[8:16, 384:512]
        return [functools.partial(job, r) for r in range(NL)]

    def mod_jobs(hs, kr):
        nr = LR * KH // (kr[1] - kr[0])

        def job(r, tok):
            rs = slice(r * nr, (r + 1) * nr)
            h = _gate(x1_s[hs, rs, kr[0]:kr[1]], tok) * (1.0 + mod(1, *kr)) + mod(0, *kr)
            h1_s[hs, rs, kr[0]:kr[1]] = h.astype(BF16)
            return fold(h)
        return [functools.partial(job, r) for r in range(T // nr)]

    def calc_piece(kr, nch):
        return tsum(calc_mod(kr, (D + kr[0], D + kr[1]), nch=nch))

    K0, K1, K2 = KP
    K01 = (0, K1[1])
    k_s[2, :, 0:HALO, :] = jnp.zeros((NC, HALO, 128), F32)
    v_s[2, :, 0:HALO, :] = jnp.zeros((NC, HALO, 128), F32)
    Ls = perm_mats() if PM0 else None
    wait('c', 'x0')
    make_sct()
    x1_s[0] = _ln(x_v[rows(0), :].astype(F32))
    wait('sa0', 'ca0')
    calc_piece(K0, 2)
    _par(mod_jobs(0, K0), [])
    wait('W0')
    perm_w(K0, Ls)
    for a in range(HB):
        qkv_part(a, 0, 2, None, [], K0)
    wait('x12')
    for a in range(HB, 3):
        qkv_part(a, 0, 2, None, [], K0)
    _par(ln0_jobs(1, 1, K0[1]), [])
    tk = []
    for a in range(3):
        qkv_part(a, 1, 3, None, tk, K0)
    _par(ln0_jobs(2, 2, K0[1]), tk[:6])
    qkv_part(0, 2, 0, None, [], K0)
    wait('W1', 'sa1', 'ca1', 'x3')
    tm = calc_piece(K1, 2)
    qkv_part(1, 2, 0, None, [], K0)
    qkv_part(2, 2, 0, None, [], K0, tm)
    perm_w(K1, None)
    td = _spread(mod_jobs(0, K1), [])
    tk = []
    qkv_part(0, 0, 2, None, tk, K1, td)
    td = _spread(mod_jobs(1, K1), [td])
    qkv_part(1, 0, 2, None, tk, K1, td)
    td = _spread(mod_jobs(2, K1), [td])
    qkv_part(2, 0, 2, None, tk, K1, td)
    for a in range(3):
        qkv_part(a, 1, 3, None, tk, K1)
    _par(ln0_jobs(3, 3, K1[1]), tk[4:])
    for a in range(3):
        qkv_part(a, 2, 0, None, [], K1)
    wait('W2', 'sa2', 'ca2')
    tm = calc_piece(K2, CH)
    qkv_part(0, 3, 1, None, [], K01)
    qkv_part(1, 3, 1, None, [], K01, tm)
    perm_w(K2, None)
    td = _spread(mod_jobs(0, K2), [])
    qkv_part(0, 0, 2, None, [], K2, td)
    td = _spread(mod_jobs(1, K2), [td])
    qkv_part(1, 0, 2, None, [], K2, td)
    td = _spread(mod_jobs(2, K2), [td])
    qkv_part(2, 0, 2, None, [], K2, td)
    td = _spread(mod_jobs(3, K2), [td])
    toks = []
    for a in range(3):
        qkv_part(a, 1, 3, 2, toks, K2, td if a == 0 else None)
    for a in range(3):
        qkv_part(a, 2, 0, 3, toks, K2)
    for a in range(2):
        qkv_part(a, 3, 1, 0, toks, K2)
    _spread(attn_jobs(2, 0, NR, first=True, thin=TH0) + attn_jobs(3, 0, A0, asl=1, thin=TH0), [None] + toks[:-TB])
    wait('wo', 'm1', *[f'w{k}_{c}' for c in range(P0) for k in (1, 2)])
    t1 = calc_mod((2 * D, 3 * D), nch=CH)
    t2 = calc_mod((4 * D, 5 * D), nch=CH, last=t1)
    t3 = calc_mod((3 * D, 4 * D), nch=CH, last=t2)
    perm_wo()
    qkv_part(2, 3, 1, 0, [], tok=tsum(t1), j1=JV)
    if WS:
        wo_mm(0, 1, [], 0, T // 2, ln=True, tok=tsum(t2))
        wo_mm(0, 1, [], T // 2, T // 2, ln=True, tok=tsum(t3))
    else:
        wo_mm(0, 1, [], ln=True, tok=tsum(t2))
    qkv_part(2, 3, 1, 0, [], j0=JV)
    f = FFN()
    toks = []
    seq0 = [s for s in SEQ if s[1] < P0]
    seq1 = [s for s in SEQ if s not in seq0]
    f.run(seq0, toks)
    _spread(attn_jobs(3, A0, A1, asl=1, thin=TH1), toks[:-3])
    wait('gb', *[f'w{k}_{c}' for c in range(P0, nch) for k in (1, 2)])
    tg = tsum(calc_mod((5 * D, 6 * D), nch=1))
    toks = []
    f.run(seq1[:-2], toks)
    _spread(attn_jobs(3, A1, NR, asl=1, thin=TH1), [None] + toks[:-4])
    wo_mm(1, 0, [], ln=True, asl=1, tok=tg)
    f.run(seq1[-2:], [])
    f.fin(0, 1)
    out_copy(0).start()
    wait('xr')
    lax.fori_loop(1, n - 3, body, 0)
    for t in (n - 3, n - 2):
        xs = (t - n + 3) & 1
        f = FFN()
        toks = []
        f.run(SEQ[:3], toks)
        if t == n - 2:
            out_copy(t - 1).start()
        f.run(SEQ[3:-2], toks)
        _spread(attn_jobs((t + 1) & 1, 0, NR, thin=TH2), toks[:-6])
        wo_mm(t + 1, 1 - xs, [], ln=True)
        f.run(SEQ[-2:], [])
        f.fin(t, xs)
    f = FFN()
    f.run(SEQ[:3], [])
    out_copy(n - 2).start()
    f.run(SEQ[3:-2], [])
    f.fin_cols(n - 1, 0)
    for t in range(n - 1):
        out_copy(t).wait()
    for j in range(NC):
        out_copy_col(n - 1, j).wait()


A0 = 0
A1 = 14
P0 = 3
HB = 2
KP = ((0, 128), (128, 256), (256, 512))
PM0 = False
TB = 8
CH = 2
LD = 4
L0 = 0
JV = 2
WS = 1
TH0 = 2
TH1 = 0
TH2 = 0


@jax.jit
def pallas_adaLN_cond__sliding_local_dilated__dense_activation_silu__prompt_kernel(
    A_x, A_wqkv, A_wo, B_x, B_w1, B_w2, c, w_mod,
):
    B, S, _ = A_x.shape
    Fd = B_w1.shape[1]
    n = S // T
    nch = Fd // FC
    x2 = A_x.reshape(S, D)
    anyspec = pl.BlockSpec(memory_space=pl.ANY)
    out = pl.pallas_call(
        functools.partial(_kernel, n=n, nch=nch),
        in_specs=[anyspec] * 7,
        out_specs=anyspec,
        out_shape=jax.ShapeDtypeStruct((S, D), A_x.dtype),
        scratch_shapes=[
            pltpu.VMEM((S, D), BF16),
            pltpu.VMEM((S, D), BF16),
            pltpu.VMEM((D, 3 * D), BF16),
            pltpu.VMEM((D, D), BF16),
            pltpu.VMEM((nch, D, FC), BF16),
            pltpu.VMEM((nch, FC, D), BF16),
            pltpu.VMEM((1, D), BF16),
            pltpu.VMEM((D, 6 * D), BF16),
            pltpu.VMEM((D // 2, 3 * D), U32),
            pltpu.VMEM((D, D), BF16),
            pltpu.VMEM((1, 6 * D), F32),
            pltpu.VMEM((D, 128), F32),
            pltpu.VMEM((SLOTS, NC, T, 128), F32),
            pltpu.VMEM((SLOTS, NC, T + HALO, 128), F32),
            pltpu.VMEM((SLOTS, NC, T + HALO, 128), F32),
            pltpu.VMEM((2, T, D), BF16),
            pltpu.VMEM((4, T, D), BF16),
            pltpu.VMEM((T, D), BF16),
            pltpu.VMEM((4, T, D), F32),
            pltpu.SemaphoreType.DMA((17 + 2 * nch,)),
            pltpu.SemaphoreType.DMA((n + NC - 1,)),
        ],
        compiler_params=pltpu.CompilerParams(vmem_limit_bytes=100 * 1024 * 1024),
    )(x2, A_wqkv, A_wo, B_w1, B_w2, c, w_mod)
    return out.reshape(B, S, D)
```

```python
import functools
import jax
import jax.numpy as jnp
from jax import lax
import jax.experimental.pallas as pl
import jax.experimental.pallas.tpu as pltpu

F32 = jnp.float32
BF16 = jnp.bfloat16
U32 = jnp.uint32
I32 = jnp.int32
H = 32
DH = 16
W = 8
DIL = 2
HALO = 16
T = 256
R = 8
D = 512
KH = D // 2
NC = D // 128
FC = 256
LR = 16
NL = T // LR
NR = T // R
SLOTS = 4
TA = 6
LOG2E = 1.4426950408889634
QSCALE = DH ** -0.5 * LOG2E


def _ln(x):
    m = jnp.mean(x, axis=-1, keepdims=True)
    xc = x - m
    v = jnp.mean(xc * xc, axis=-1, keepdims=True)
    return xc * lax.rsqrt(v + 1e-5)


def _silu(u):
    return u * (0.5 * jnp.tanh(0.5 * u) + 0.5)


def _zero_of(tok):
    z = pltpu.bitcast(tok, U32)
    return lax.shift_right_logical(lax.shift_right_logical(z, U32(16)), U32(16))


def _gate(v, tok):
    if tok is None:
        return v
    z = _zero_of(tok)
    u = pltpu.bitcast(v, U32)
    reps = (u.shape[0] // 8, u.shape[1] // 128)
    zz = z if reps == (1, 1) else jnp.tile(z, reps)
    return pltpu.bitcast(u | zz, v.dtype)


def _spread(jobs, toks):
    extra = None
    for k, job in enumerate(jobs):
        tok = toks[k * len(toks) // len(jobs)] if toks else None
        if extra is not None:
            tok = extra if tok is None else tok + extra
        extra = job(tok)
    return extra


def _par(jobs, toks):
    out = None
    for k, job in enumerate(jobs):
        r = job(toks[k * len(toks) // len(jobs)] if toks else None)
        out = r if out is None else out + r
    return out


def _merge(a, b):
    out = []
    j = 0
    for i, x in enumerate(a):
        out.append(x)
        while j < len(b) and (j + 1) * len(a) <= (i + 1) * (len(b) + 1) and j < len(b):
            out.append(b[j])
            j += 1
    out.extend(b[j:])
    return out


def _kernel(*refs, n, nch):
    pl.run_scoped(lambda sem: _main(*refs, sem, n=n, nch=nch), pltpu.SemaphoreType.DMA((6,)))
    o_hbm, o_v, sem_out = refs[7], refs[9], refs[-1]
    pltpu.make_async_copy(o_v, o_hbm, sem_out.at[0]).wait()


def _main(x_hbm, wqkv_hbm, wo_hbm, w1_hbm, w2_hbm, c_hbm, wmod_hbm, o_hbm,
            x_v, o_v, wqkv_v, wo_v, w1_v, w2_v, c_v, wmod_v,
            wqkv_p, wo_p, wo_f, mod_ref, sct, q_s, k_s, v_s, a_s, h1_s, h2_s, x1_s,
            sem_out, sem, *, n, nch):
    cps = {}

    def add(name, src, dst, si):
        cps[name] = pltpu.make_async_copy(src, dst, sem.at[si])
        cps[name].start()

    def xt(a, b):
        return x_hbm.at[pl.ds(a * T, (b - a) * T)], x_v.at[pl.ds(a * T, (b - a) * T)]

    def mcols(c0, nc):
        return wmod_hbm.at[:, pl.ds(c0, nc)], wmod_v.at[:, pl.ds(c0, nc)]

    def piece(i, sm, sw):
        k0, k1 = KP[i]
        add(f'sa{i}', *mcols(k0, k1 - k0), sm)
        add(f'ca{i}', *mcols(D + k0, k1 - k0), sm)
        add(f'W{i}', wqkv_hbm.at[pl.ds(k0, k1 - k0)], wqkv_v.at[pl.ds(k0, k1 - k0)], sw)

    def pairs(c0, c1, si):
        for c in range(c0, c1):
            add(f'w1_{c}', w1_hbm.at[:, pl.ds(c * FC, FC)], w1_v.at[c], si)
            add(f'w2_{c}', w2_hbm.at[pl.ds(c * FC, FC)], w2_v.at[c], si)

    def x_late(t):
        return pltpu.make_async_copy(x_hbm.at[rows(t)], x_v.at[rows(t)], sem.at[t - 2])

    add('c', c_hbm, c_v, 0)
    add('x0', *xt(0, 1), 0)
    piece(0, 1, 2)
    add('x12', *xt(1, 3), 3)
    piece(1, 4, 4)
    add('x3', *xt(3, 4), 4)
    add('wo', wo_hbm, wo_v, 5)
    piece(2, 5, 5)

    def wait(*names):
        for name in names:
            cps[name].wait()

    def mod(k, c0=0, c1=D):
        return mod_ref[0:1, k * D + c0:k * D + c1]

    def rows(t, r0=0, nr=T):
        if isinstance(t, int):
            return pl.ds(t * T + r0, nr)
        return pl.ds(pl.multiple_of(t * T + r0, nr), nr)

    def make_sct():
        c = c_v[...].astype(F32)
        sc = (c * jax.nn.sigmoid(c)).astype(BF16).astype(F32)
        r = lax.broadcasted_iota(I32, (128, 128), 0)
        l = lax.broadcasted_iota(I32, (128, 128), 1)
        ones = jnp.ones((128, 128), BF16)
        for b in range(NC):
            dg = jnp.where(r == l, sc[:, b * 128:(b + 1) * 128], 0.0).astype(BF16)
            sct[b * 128:(b + 1) * 128, :] = jnp.dot(dg, ones, preferred_element_type=F32)

    def calc_mod(*rngs, nch=2, last=None):
        blocks = [c for c0, c1 in rngs for c in range(c0, c1, 128)]
        last = [None] * nch if last is None else list(last)
        for b0 in range(0, len(blocks), nch):
            grp = blocks[b0:b0 + nch]
            acc = [None] * len(grp)
            for g in range(D // 16):
                s = sct[g * 16:(g + 1) * 16, :]
                for bi, c in enumerate(grp):
                    p = wmod_v[g * 16:(g + 1) * 16, c:c + 128].astype(F32) * s
                    a = _gate(p[0:8], last[bi]) if acc[bi] is None else acc[bi] + p[0:8]
                    acc[bi] = a + p[8:16]
            for bi, c in enumerate(grp):
                mod_ref[0:1, c:c + 128] = jnp.sum(acc[bi], axis=0, keepdims=True)
                last[bi] = acc[bi]
        return last

    def tsum(ts):
        return functools.reduce(lambda u, v: u + v, ts)

    def perm_mats():
        src = lax.broadcasted_iota(I32, (128, 128), 0)
        m = lax.broadcasted_iota(I32, (128, 128), 1)
        out = []
        for i in range(NC):
            j = ((m >> 3) + (4 - i)) & 3
            l = (m + 128 - 8 * j) & 127
            out.append(jnp.where(src == (m & 7) * 16 + 4 * j + (l >> 5), 1.0, 0.0).astype(BF16))
        return out

    def perm_w(kr, Ls):
        rs = slice(kr[0], kr[1])
        ru = slice(kr[0] // 2, kr[1] // 2)
        m = lax.broadcasted_iota(I32, ((kr[1] - kr[0]) // 2, 128), 1)
        g = (m >> 3) & 3
        for a in range(3):
            wp = []
            for i in range(NC):
                w = wqkv_v[rs, a * D + i * 128:a * D + (i + 1) * 128]
                if Ls is None:
                    j = ((m >> 3) + (4 - i)) & 3
                    l = (m + 128 - 8 * j) & 127
                    idx = (m & 7) * 16 + 4 * j + (l >> 5)
                    wp.append(jnp.take_along_axis(pltpu.bitcast(w, U32), idx, axis=1))
                else:
                    wp.append(pltpu.bitcast(
                        jnp.dot(w, Ls[i], preferred_element_type=F32).astype(BF16), U32))
            for j in range(NC):
                pre = wp[(3 - j) % 4]
                for gg in (2, 1, 0):
                    pre = jnp.where(g == gg, wp[(gg - j) % 4], pre)
                if j:
                    pre = pltpu.roll(pre, 128 - 8 * j, 1)
                wqkv_p[ru, a * D + j * 128:a * D + (j + 1) * 128] = pre

    def wq(ks, c0, c1):
        return pltpu.bitcast(wqkv_p[ks.start // 2:ks.stop // 2, c0:c1], BF16)

    def perm_wo_jobs():
        def cvt(j, r0, tok):
            w = _gate(wo_v[r0:r0 + 128, j * 128:(j + 1) * 128], tok).astype(F32)
            for h in range(128 // DH):
                wo_f[j, pl.ds(r0 // DH + h, DH, stride=SS), :] = w[h * DH:(h + 1) * DH]
            return w[120:128]

        def mov(j, d, tok):
            w = _gate(wo_f[j, d * SS:d * SS + H, :], tok)
            wo_p[d * H:(d + 1) * H, j * 128:(j + 1) * 128] = w.astype(BF16)
            return w[24:32]
        cv = [[functools.partial(cvt, j, r0) for r0 in range(0, D, 128)] for j in range(NC)]
        out = cv[0]
        for j in range(NC):
            out = out + _merge([functools.partial(mov, j, d) for d in range(DH)], cv[j + 1] if j + 1 < NC else [])
        return out

    def ln1_jobs(t, hs, chain=False):
        def job(r, tok):
            x = _gate(x_v[rows(t, r * LR, LR), :], tok).astype(F32)
            h = _ln(x) * (1.0 + mod(1)) + mod(0)
            h1_s[hs, r * LR:(r + 1) * LR, :] = h.astype(BF16)
            if chain:
                return h[0:8, 0:128] + h[8:16, 0:128]
        return [functools.partial(job, r) for r in range(NL)]

    def ln2_jobs(xs, r0=0, r1=NL):
        def job(r, tok):
            x1 = _gate(x1_s[xs, r * LR:(r + 1) * LR, :], tok)
            h2_s[r * LR:(r + 1) * LR, :] = (_ln(x1) * (1.0 + mod(4)) + mod(3)).astype(BF16)
        return [functools.partial(job, r) for r in range(r0, r1)]

    def tok_of(v, toks, cbs, nr=2):
        for cb in cbs:
            for row in range(0, v.shape[0], v.shape[0] // nr):
                toks.append(v[row:row + 8, cb * 128:(cb + 1) * 128])

    def gate_rows(w, tok):
        if tok is None:
            return w
        pcs = []
        for k0 in range(0, w.shape[0], 128):
            pcs += [_gate(w[k0:k0 + 16], tok), w[k0 + 16:k0 + 128]]
        return jnp.concatenate(pcs, axis=0)

    def qkv_part(a, hs, sl, prev, toks, kr=(0, D), tok=None, j0=0, j1=NC):
        dst = (q_s, k_s, v_s)[a]
        if a and prev is not None:
            dst[sl, j0:j1, 0:HALO, :] = dst[prev, j0:j1, T:T + HALO, :]
        ks = slice(*kr)
        r = jnp.dot(h1_s[hs, :, ks], gate_rows(wq(ks, a * D + j0 * 128, a * D + j1 * 128), tok),
                    preferred_element_type=F32)
        tok_of(r, toks, range(0, j1 - j0, D // (kr[1] - kr[0])), 4)
        o = 0 if a == 0 else HALO
        for j in range(j0, j1):
            rj = r[:, (j - j0) * 128:(j - j0 + 1) * 128]
            if kr[0]:
                rj = rj + dst[sl, j, o:o + T, :]
            if a == 0 and kr[1] == D:
                rj = rj * QSCALE
            dst[sl, j, o:o + T, :] = rj

    def attn_jobs(sl, ra, rb, first=False, asl=0, thin=0, ret=False):
        last = [None] * max(thin, 1)

        def job(r, tok):
            r0 = r * R
            q = [_gate(q_s[sl, j, r0:r0 + R, :], tok) for j in range(NC)]
            logits = []
            for w in range(W):
                s0 = HALO + r0 - DIL * w
                tt = q[0] * k_s[sl, 0, s0:s0 + R, :]
                for j in range(1, NC):
                    tt = tt + q[j] * k_s[sl, j, s0:s0 + R, :]
                tt = tt + pltpu.roll(tt, 64, 1)
                tt = tt + pltpu.roll(tt, 32, 1)
                if first and r0 < HALO and w > 0:
                    row = r0 + lax.broadcasted_iota(I32, (R, 128), 0)
                    tt = jnp.where(row >= DIL * w, tt, -1e9 * LOG2E)
                logits.append(tt)
            m = logits[0]
            for w in range(1, W):
                m = jnp.maximum(m, logits[w])
            ps = [jnp.exp2(l - m) for l in logits]
            den = ps[0]
            for w in range(1, W):
                den = den + ps[w]
            inv = 1.0 / den
            res = None
            for j in range(NC):
                acc = None
                for w in range(W):
                    s0 = HALO + r0 - DIL * w
                    term = ps[w] * v_s[sl, j, s0:s0 + R, :]
                    if acc is None:
                        acc = _gate(term, last[j % thin]) if thin else term
                    else:
                        acc = acc + term
                if thin:
                    last[j % thin] = acc
                o = acc * inv
                res = o if res is None else res + o
                a_s[asl, r0:r0 + R, j * 128:(j + 1) * 128] = o.astype(BF16)
            if ret:
                return res
        return [functools.partial(job, r) for r in range(ra, rb)]

    def wo_mm(t, xs, toks, r0=0, nr=T, ln=False, asl=0, tok=None):
        att = jnp.dot(a_s[asl, r0:r0 + nr, :], gate_rows(wo_p[...], tok), preferred_element_type=F32)
        tok_of(att, toks, range(NC))
        x1 = x_v[rows(t, r0, nr), :].astype(F32) + mod(2) * att
        x1_s[xs, r0:r0 + nr, :] = x1
        if ln:
            h2_s[r0:r0 + nr, :] = (_ln(x1) * (1.0 + mod(4)) + mod(3)).astype(BF16)

    def out_copy(t):
        return pltpu.make_async_copy(o_v.at[rows(t)], o_hbm.at[rows(t)], sem_out.at[0])

    def out_copy_col(t, j, r0=0, nr=T):
        cs = pl.ds(j * 128, 128)
        return pltpu.make_async_copy(o_v.at[rows(t, r0, nr), cs], o_hbm.at[rows(t, r0, nr), cs], sem_out.at[0])

    class FFN:
        def __init__(self):
            self.us = []
            self.y = None

        def w1(self, c, toks, split=False):
            if split:
                u = jnp.concatenate([
                    jnp.dot(h2_s[hh * (T // 2):(hh + 1) * (T // 2), :], w1_v[c], preferred_element_type=F32)
                    for hh in range(2)], axis=0)
            else:
                u = jnp.dot(h2_s[...], w1_v[c], preferred_element_type=F32)
            tok_of(u, toks, range(FC // 128))
            self.us.append(_silu(u).astype(BF16))

        def w2(self, c, toks):
            p = jnp.dot(self.us[c], w2_v[c], preferred_element_type=F32)
            tok_of(p, toks, (0, 2))
            self.y = p if self.y is None else self.y + p

        def run(self, seq, toks):
            for kind, c in seq:
                (self.w1 if kind == 1 else self.w2)(c, toks)

        def fin(self, t, xs):
            o_v[rows(t), :] = (x1_s[xs] + mod(5) * self.y).astype(BF16)

        def fin_cols(self, t, xs):
            uu = jnp.concatenate(self.us[nch - 2:], axis=1)
            for j in range(NC):
                cs = slice(j * 128, (j + 1) * 128)
                wj = jnp.concatenate([w2_v[nch - 2, :, cs], w2_v[nch - 1, :, cs]], axis=0)
                y = self.y[:, cs] + jnp.dot(uu, wj, preferred_element_type=F32)
                o = (x1_s[xs, :, cs] + mod(5, j * 128, (j + 1) * 128) * y).astype(BF16)
                for r0, nr in ((0, T - LS), (T - LS, LS)) if (LS and j == NC - 1) else ((0, T),):
                    o_v[rows(t, r0, nr), cs] = o[r0:r0 + nr]
                    out_copy_col(t, j, r0, nr).start()

    SEQ = [(1, 0)]
    for c in range(nch):
        if c + 1 < nch:
            SEQ.append((1, c + 1))
        SEQ.append((2, c))

    def body(t, carry):
        sl = (t + 1) & 1
        x_late(t + 3).wait()
        f = FFN()
        toks = []
        f.run(SEQ, toks)
        _spread(_merge(attn_jobs(sl, 0, NR, thin=TH2), ln1_jobs(t + 3, 0, True)), toks[:len(toks) - TA])
        f.fin(t, 0)
        wo_mm(t + 1, 0, [], ln=True)
        for a in range(3):
            qkv_part(a, 0, sl, 1 - sl, [])
        out_copy(t).start()
        return carry

    def fold(h):
        parts = [h[r:r + 8, c:c + 128] for r in range(0, h.shape[0], 8) for c in range(0, h.shape[1], 128)]
        return tsum(parts)

    def ln0_jobs(t, hs, k1):
        def job(r, tok):
            rs = slice(r * LR, (r + 1) * LR)
            y = _ln(_gate(x_v[rows(t, r * LR, LR), :], tok).astype(F32))
            x1_s[hs, rs, k1:] = y[:, k1:]
            h = y[:, :k1] * (1.0 + mod(1, 0, k1)) + mod(0, 0, k1)
            h1_s[hs, rs, :k1] = h.astype(BF16)
            return h[0:8, 0:128] + h[8:16, 0:128] + y[0:8, 256:384] + y[8:16, 384:512]
        return [functools.partial(job, r) for r in range(NL)]

    def mod_jobs(hs, kr):
        nr = LR * KH // (kr[1] - kr[0])

        def job(r, tok):
            rs = slice(r * nr, (r + 1) * nr)
            h = _gate(x1_s[hs, rs, kr[0]:kr[1]], tok) * (1.0 + mod(1, *kr)) + mod(0, *kr)
            h1_s[hs, rs, kr[0]:kr[1]] = h.astype(BF16)
            return fold(h)
        return [functools.partial(job, r) for r in range(T // nr)]

    def calc_piece(kr, nch):
        return tsum(calc_mod(kr, (D + kr[0], D + kr[1]), nch=nch))

    K0, K1, K2 = KP
    K01 = (0, K1[1])
    k_s[2, :, 0:HALO, :] = jnp.zeros((NC, HALO, 128), F32)
    v_s[2, :, 0:HALO, :] = jnp.zeros((NC, HALO, 128), F32)
    Ls = perm_mats() if PM0 else None
    wait('c', 'x0')
    add('m1', *mcols(2 * D, 3 * D), 0)
    pairs(0, P0, 0)
    make_sct()
    x1_s[0] = _ln(x_v[rows(0), :].astype(F32))
    wait('sa0', 'ca0')
    add('gb', *mcols(5 * D, D), 1)
    pairs(P0, nch, 1)
    calc_piece(K0, 2)
    _par(mod_jobs(0, K0), [])
    wait('W0')
    x_late(4).start()
    perm_w(K0, Ls)
    for a in range(HB):
        qkv_part(a, 0, 2, None, [], K0)
    wait('x12')
    x_late(5).start()
    for a in range(HB, 3):
        qkv_part(a, 0, 2, None, [], K0)
    _par(ln0_jobs(1, 1, K0[1]), [])
    tk = []
    for a in range(3):
        qkv_part(a, 1, 3, None, tk, K0)
    _par(ln0_jobs(2, 2, K0[1]), tk[:6])
    for a in range(HB4):
        qkv_part(a, 2, 0, None, [], K0)
    wait('W1', 'sa1', 'ca1', 'x3')
    x_late(6).start()
    tm = calc_piece(K1, 2)
    for a in range(HB4, 3):
        qkv_part(a, 2, 0, None, [], K0, tm if (a == 2 and HB4 < 2) else None)
    perm_w(K1, None)
    td = _spread(mod_jobs(0, K1), [])
    tk = []
    qkv_part(0, 0, 2, None, tk, K1, td)
    td = _spread(mod_jobs(1, K1), [td])
    qkv_part(1, 0, 2, None, tk, K1, td)
    td = _spread(mod_jobs(2, K1), [td])
    qkv_part(2, 0, 2, None, tk, K1, td)
    for a in range(3):
        qkv_part(a, 1, 3, None, tk, K1)
    _par(ln0_jobs(3, 3, K1[1]), tk[4:])
    for a in range(3):
        qkv_part(a, 2, 0, None, [], K1)
    qkv_part(2, 3, 1, None, [], K01)
    if QB:
        qkv_part(0, 3, 1, None, [], K01, j1=QB)
    wait('W2', 'sa2', 'ca2', 'wo')
    x_late(7).start()
    tm = calc_piece(K2, CH)
    if QB < NC:
        qkv_part(0, 3, 1, None, [], K01, j0=QB)
    qkv_part(1, 3, 1, None, [], K01, tm if QB == 0 else None)
    perm_w(K2, None)
    td = _spread(mod_jobs(0, K2), [])
    tk = []
    qkv_part(0, 0, 2, None, tk, K2, td)
    td = _spread(mod_jobs(1, K2), [td])
    qkv_part(1, 0, 2, None, tk, K2, td)
    td = _spread(mod_jobs(2, K2), [td])
    qkv_part(2, 0, 2, None, tk, K2, td)
    td = _spread(mod_jobs(3, K2), [td])
    dots = [(a, 1, 3, 2) for a in range(3)] + [(a, 2, 0, 3) for a in range(3)] + [(a, 3, 1, 0) for a in range(2)]
    jobs = attn_jobs(2, 0, NR, first=True, thin=TH0, ret=True)
    L = [None] + tk[AV:]
    nL = len(L) + 8 * len(dots) - TB
    pj = perm_wo_jobs()
    off = PW0 - AV + 1
    done = []
    k = kp = 0
    for i in range(len(dots) + 1):
        res = []
        while k < NR and k * nL // NR < len(L):
            res.append(jobs[k](L[k * nL // NR]))
            k += 1
        while kp < len(pj) and off + kp * (PW1 - PW0) // len(pj) < len(L):
            q = off + kp * (PW1 - PW0) // len(pj)
            r = pj[kp](L[q] if q > 0 else tk[q + AV - 1])
            if PD:
                res.append(r)
            kp += 1
        done.append(tsum(res) if res else None)
        if i < len(dots):
            g = td if i == 0 else (done[i - DL] if i >= DL else None)
            qkv_part(*dots[i], L, K2, g)
    wait('m1', *[f'w{k}_{c}' for c in range(P0) for k in (1, 2)])
    t1 = calc_mod((2 * D, 3 * D), nch=CH1)
    t2 = calc_mod((4 * D, 5 * D), nch=CH1, last=t1)
    t3 = calc_mod((3 * D, 4 * D), nch=CH1, last=t2)
    gs = [None, tsum(t1), tsum(t2), tsum(t3)]
    wo_mm(0, 1, [], 0, T // 2, ln=True)
    wo_mm(0, 1, [], T // 2, T // 2, ln=True, tok=gs[G1])
    qkv_part(2, 3, 1, 0, [], K2, tok=gs[G2])
    f = FFN()
    toks = []
    seq0 = [s for s in SEQ if s[1] < P0]
    seq1 = [s for s in SEQ if s not in seq0]
    f.run(seq0, toks)
    _spread(attn_jobs(3, A0, A1, asl=1, thin=TH1), toks[:-3])
    wait('gb', *[f'w{k}_{c}' for c in range(P0, nch) for k in (1, 2)])
    tg = tsum(calc_mod((5 * D, 6 * D), nch=1))
    toks = []
    f.run(seq1[:-2], toks)
    _spread(attn_jobs(3, A1, NR, asl=1, thin=TH1), [None] + toks[:-4])
    wo_mm(1, 0, [], ln=True, asl=1, tok=tg)
    f.run(seq1[-2:], [])
    f.fin(0, 1)
    out_copy(0).start()
    lax.fori_loop(1, n - 3, body, 0)
    for t in (n - 3, n - 2):
        xs = (t - n + 3) & 1
        f = FFN()
        toks = []
        f.run(SEQ[:3], toks)
        if t == n - 2:
            out_copy(t - 1).start()
        f.run(SEQ[3:-2], toks)
        _spread(attn_jobs((t + 1) & 1, 0, NR, thin=TH2), toks[:-6])
        wo_mm(t + 1, 1 - xs, [], ln=True)
        f.run(SEQ[-2:], [])
        f.fin(t, xs)
    f = FFN()
    f.run(SEQ[:3], [])
    out_copy(n - 2).start()
    f.run(SEQ[3:-2], [])
    f.fin_cols(n - 1, 0)


A0 = 0
A1 = 14
P0 = 3
HB = 2
KP = ((0, 128), (128, 256), (256, 512))
PM0 = False
TB = 10
CH = 2
LD = 4
L0 = 0
JV = 2
LS = 128
WF = 0
HB4 = 1
QB = 2
PD = 0
DL = 1
AV = 16
SS = 33
PW0 = 8
PW1 = 80
CH1 = 2
G1 = 1
G2 = 3
WS = 1
TH0 = 2
TH1 = 0
TH2 = 0


@jax.jit
def pallas_adaLN_cond__sliding_local_dilated__dense_activation_silu__prompt_kernel(
    A_x, A_wqkv, A_wo, B_x, B_w1, B_w2, c, w_mod,
):
    B, S, _ = A_x.shape
    Fd = B_w1.shape[1]
    n = S // T
    nch = Fd // FC
    assert n == 8
    x2 = A_x.reshape(S, D)
    anyspec = pl.BlockSpec(memory_space=pl.ANY)
    out = pl.pallas_call(
        functools.partial(_kernel, n=n, nch=nch),
        in_specs=[anyspec] * 7,
        out_specs=anyspec,
        out_shape=jax.ShapeDtypeStruct((S, D), A_x.dtype),
        scratch_shapes=[
            pltpu.VMEM((S, D), BF16),
            pltpu.VMEM((S, D), BF16),
            pltpu.VMEM((D, 3 * D), BF16),
            pltpu.VMEM((D, D), BF16),
            pltpu.VMEM((nch, D, FC), BF16),
            pltpu.VMEM((nch, FC, D), BF16),
            pltpu.VMEM((1, D), BF16),
            pltpu.VMEM((D, 6 * D), BF16),
            pltpu.VMEM((D // 2, 3 * D), U32),
            pltpu.VMEM((D, D), BF16),
            pltpu.VMEM((NC, DH * 40, 128), F32),
            pltpu.VMEM((1, 6 * D), F32),
            pltpu.VMEM((D, 128), F32),
            pltpu.VMEM((SLOTS, NC, T, 128), F32),
            pltpu.VMEM((SLOTS, NC, T + HALO, 128), F32),
            pltpu.VMEM((SLOTS, NC, T + HALO, 128), F32),
            pltpu.VMEM((2, T, D), BF16),
            pltpu.VMEM((4, T, D), BF16),
            pltpu.VMEM((T, D), BF16),
            pltpu.VMEM((4, T, D), F32),
            pltpu.SemaphoreType.DMA((1,)),
        ],
        compiler_params=pltpu.CompilerParams(vmem_limit_bytes=100 * 1024 * 1024),
    )(x2, A_wqkv, A_wo, B_w1, B_w2, c, w_mod)
    return out.reshape(B, S, D)
```

```python
import functools
import jax
import jax.numpy as jnp
from jax import lax
import jax.experimental.pallas as pl
import jax.experimental.pallas.tpu as pltpu

F32 = jnp.float32
BF16 = jnp.bfloat16
U32 = jnp.uint32
I32 = jnp.int32
H = 32
DH = 16
W = 8
DIL = 2
HALO = 16
T = 256
R = 8
D = 512
KH = D // 2
NC = D // 128
FC = 256
LR = 16
NL = T // LR
NR = T // R
SLOTS = 4
TA = 6
LOG2E = 1.4426950408889634
QSCALE = DH ** -0.5 * LOG2E


def _ln(x):
    m = jnp.mean(x, axis=-1, keepdims=True)
    xc = x - m
    v = jnp.mean(xc * xc, axis=-1, keepdims=True)
    return xc * lax.rsqrt(v + 1e-5)


def _silu(u):
    return u * (0.5 * jnp.tanh(0.5 * u) + 0.5)


def _zero_of(tok):
    z = pltpu.bitcast(tok, U32)
    return lax.shift_right_logical(lax.shift_right_logical(z, U32(16)), U32(16))


def _gate(v, tok):
    if tok is None:
        return v
    z = _zero_of(tok)
    u = pltpu.bitcast(v, U32)
    reps = (u.shape[0] // 8, u.shape[1] // 128)
    zz = z if reps == (1, 1) else jnp.tile(z, reps)
    return pltpu.bitcast(u | zz, v.dtype)


def _spread(jobs, toks):
    extra = None
    for k, job in enumerate(jobs):
        tok = toks[k * len(toks) // len(jobs)] if toks else None
        if extra is not None:
            tok = extra if tok is None else tok + extra
        extra = job(tok)
    return extra


def _par(jobs, toks):
    out = None
    for k, job in enumerate(jobs):
        r = job(toks[k * len(toks) // len(jobs)] if toks else None)
        out = r if out is None else out + r
    return out


def _merge(a, b):
    out = []
    j = 0
    for i, x in enumerate(a):
        out.append(x)
        while j < len(b) and (j + 1) * len(a) <= (i + 1) * (len(b) + 1) and j < len(b):
            out.append(b[j])
            j += 1
    out.extend(b[j:])
    return out


def _kernel(*refs, n, nch):
    pl.run_scoped(lambda sem: _main(*refs, sem, n=n, nch=nch), pltpu.SemaphoreType.DMA((6,)))
    o_hbm, o_v, sem_out = refs[7], refs[9], refs[-1]
    pltpu.make_async_copy(o_v, o_hbm, sem_out.at[0]).wait()


def _main(x_hbm, wqkv_hbm, wo_hbm, w1_hbm, w2_hbm, c_hbm, wmod_hbm, o_hbm,
            x_v, o_v, wqkv_v, wo_v, w1_v, w2_v, c_v, wmod_v,
            wqkv_p, wo_p, wo_f, mod_ref, sct, q_s, k_s, v_s, a_s, h1_s, h2_s, x1_s,
            sem_out, sem, *, n, nch):
    cps = {}

    def add(name, src, dst, si):
        cps[name] = pltpu.make_async_copy(src, dst, sem.at[si])
        cps[name].start()

    def xt(a, b):
        return x_hbm.at[pl.ds(a * T, (b - a) * T)], x_v.at[pl.ds(a * T, (b - a) * T)]

    def mcols(c0, nc):
        return wmod_hbm.at[:, pl.ds(c0, nc)], wmod_v.at[:, pl.ds(c0, nc)]

    def piece(i, sm, sw):
        k0, k1 = KP[i]
        add(f'sa{i}', *mcols(k0, k1 - k0), sm)
        add(f'ca{i}', *mcols(D + k0, k1 - k0), sm)
        add(f'W{i}', wqkv_hbm.at[pl.ds(k0, k1 - k0)], wqkv_v.at[pl.ds(k0, k1 - k0)], sw)

    def pairs(c0, c1, si):
        for c in range(c0, c1):
            add(f'w1_{c}', w1_hbm.at[:, pl.ds(c * FC, FC)], w1_v.at[c], si)
            add(f'w2_{c}', w2_hbm.at[pl.ds(c * FC, FC)], w2_v.at[c], si)

    def x_late(t):
        return pltpu.make_async_copy(x_hbm.at[rows(t)], x_v.at[rows(t)], sem.at[t - 2])

    add('c', c_hbm, c_v, 0)
    add('x0', *xt(0, 1), 0)
    piece(0, 1, 2)
    add('x12', *xt(1, 3), 3)
    piece(1, 4, 4)
    add('x3', *xt(3, 4), 4)
    add('wo', wo_hbm, wo_v, 5)
    piece(2, 5, 5)

    def wait(*names):
        for name in names:
            cps[name].wait()

    def mod(k, c0=0, c1=D):
        return mod_ref[0:1, k * D + c0:k * D + c1]

    def rows(t, r0=0, nr=T):
        if isinstance(t, int):
            return pl.ds(t * T + r0, nr)
        return pl.ds(pl.multiple_of(t * T + r0, nr), nr)

    def make_sct():
        c = c_v[...].astype(F32)
        sc = (c * jax.nn.sigmoid(c)).astype(BF16).astype(F32)
        r = lax.broadcasted_iota(I32, (128, 128), 0)
        l = lax.broadcasted_iota(I32, (128, 128), 1)
        ones = jnp.ones((128, 128), BF16)
        for b in range(NC):
            dg = jnp.where(r == l, sc[:, b * 128:(b + 1) * 128], 0.0).astype(BF16)
            sct[b * 128:(b + 1) * 128, :] = jnp.dot(dg, ones, preferred_element_type=F32)

    def calc_mod(*rngs, nch=2, last=None):
        blocks = [c for c0, c1 in rngs for c in range(c0, c1, 128)]
        last = [None] * nch if last is None else list(last)
        for b0 in range(0, len(blocks), nch):
            grp = blocks[b0:b0 + nch]
            acc = [None] * len(grp)
            for g in range(D // 16):
                s = sct[g * 16:(g + 1) * 16, :]
                for bi, c in enumerate(grp):
                    p = wmod_v[g * 16:(g + 1) * 16, c:c + 128].astype(F32) * s
                    a = _gate(p[0:8], last[bi]) if acc[bi] is None else acc[bi] + p[0:8]
                    acc[bi] = a + p[8:16]
            for bi, c in enumerate(grp):
                mod_ref[0:1, c:c + 128] = jnp.sum(acc[bi], axis=0, keepdims=True)
                last[bi] = acc[bi]
        return last

    def tsum(ts):
        return functools.reduce(lambda u, v: u + v, ts)

    def perm_w(kr):
        rs = slice(kr[0], kr[1])
        ru = slice(kr[0] // 2, kr[1] // 2)
        m = lax.broadcasted_iota(I32, ((kr[1] - kr[0]) // 2, 128), 1)
        g = (m >> 3) & 3
        for a in range(3):
            wp = []
            for i in range(NC):
                w = wqkv_v[rs, a * D + i * 128:a * D + (i + 1) * 128]
                j = ((m >> 3) + (4 - i)) & 3
                l = (m + 128 - 8 * j) & 127
                idx = (m & 7) * 16 + 4 * j + (l >> 5)
                wp.append(jnp.take_along_axis(pltpu.bitcast(w, U32), idx, axis=1))
            for j in range(NC):
                pre = wp[(3 - j) % 4]
                for gg in (2, 1, 0):
                    pre = jnp.where(g == gg, wp[(gg - j) % 4], pre)
                if j:
                    pre = pltpu.roll(pre, 128 - 8 * j, 1)
                wqkv_p[ru, a * D + j * 128:a * D + (j + 1) * 128] = pre

    def wq(ks, c0, c1):
        return pltpu.bitcast(wqkv_p[ks.start // 2:ks.stop // 2, c0:c1], BF16)

    def perm_wo_jobs():
        def cvt(j, r0, tok):
            w = _gate(wo_v[r0:r0 + 128, j * 128:(j + 1) * 128], tok).astype(F32)
            for h in range(128 // DH):
                wo_f[j, pl.ds(r0 // DH + h, DH, stride=SS), :] = w[h * DH:(h + 1) * DH]
            return w[120:128]

        def mov(j, d, tok):
            w = _gate(wo_f[j, d * SS:d * SS + H, :], tok)
            wo_p[d * H:(d + 1) * H, j * 128:(j + 1) * 128] = w.astype(BF16)
            return w[24:32]
        cv = [[functools.partial(cvt, j, r0) for r0 in range(0, D, 128)] for j in range(NC)]
        out = cv[0]
        for j in range(NC):
            out = out + _merge([functools.partial(mov, j, d) for d in range(DH)], cv[j + 1] if j + 1 < NC else [])
        return out

    def ln1_jobs(t, hs, chain=False):
        def job(r, tok):
            x = _gate(x_v[rows(t, r * LR, LR), :], tok).astype(F32)
            h = _ln(x) * (1.0 + mod(1)) + mod(0)
            h1_s[hs, r * LR:(r + 1) * LR, :] = h.astype(BF16)
            if chain:
                return h[0:8, 0:128] + h[8:16, 0:128]
        return [functools.partial(job, r) for r in range(NL)]

    def tok_of(v, toks, cbs, nr=2):
        for cb in cbs:
            for row in range(0, v.shape[0], v.shape[0] // nr):
                toks.append(v[row:row + 8, cb * 128:(cb + 1) * 128])

    def gate_rows(w, tok):
        if tok is None:
            return w
        pcs = []
        for k0 in range(0, w.shape[0], 128):
            pcs += [_gate(w[k0:k0 + 16], tok), w[k0 + 16:k0 + 128]]
        return jnp.concatenate(pcs, axis=0)

    def qkv_part(a, hs, sl, prev, toks, kr=(0, D), tok=None, j0=0, j1=NC):
        dst = (q_s, k_s, v_s)[a]
        if a and prev is not None:
            dst[sl, j0:j1, 0:HALO, :] = dst[prev, j0:j1, T:T + HALO, :]
        ks = slice(*kr)
        r = jnp.dot(h1_s[hs, :, ks], gate_rows(wq(ks, a * D + j0 * 128, a * D + j1 * 128), tok),
                    preferred_element_type=F32)
        tok_of(r, toks, range(0, j1 - j0, D // (kr[1] - kr[0])), 4)
        o = 0 if a == 0 else HALO
        for j in range(j0, j1):
            rj = r[:, (j - j0) * 128:(j - j0 + 1) * 128]
            if kr[0]:
                rj = rj + dst[sl, j, o:o + T, :]
            if a == 0 and kr[1] == D:
                rj = rj * QSCALE
            dst[sl, j, o:o + T, :] = rj

    def attn_jobs(sl, ra, rb, first=False, asl=0, thin=0, ret=False):
        last = [None] * max(thin, 1)

        def job(r, tok):
            r0 = r * R
            q = [_gate(q_s[sl, j, r0:r0 + R, :], tok) for j in range(NC)]
            logits = []
            for w in range(W):
                s0 = HALO + r0 - DIL * w
                tt = q[0] * k_s[sl, 0, s0:s0 + R, :]
                for j in range(1, NC):
                    tt = tt + q[j] * k_s[sl, j, s0:s0 + R, :]
                tt = tt + pltpu.roll(tt, 64, 1)
                tt = tt + pltpu.roll(tt, 32, 1)
                if first and r0 < HALO and w > 0:
                    row = r0 + lax.broadcasted_iota(I32, (R, 128), 0)
                    tt = jnp.where(row >= DIL * w, tt, -1e9 * LOG2E)
                logits.append(tt)
            m = logits[0]
            for w in range(1, W):
                m = jnp.maximum(m, logits[w])
            ps = [jnp.exp2(l - m) for l in logits]
            den = ps[0]
            for w in range(1, W):
                den = den + ps[w]
            inv = 1.0 / den
            res = None
            for j in range(NC):
                acc = None
                for w in range(W):
                    s0 = HALO + r0 - DIL * w
                    term = ps[w] * v_s[sl, j, s0:s0 + R, :]
                    if acc is None:
                        acc = _gate(term, last[j % thin]) if thin else term
                    else:
                        acc = acc + term
                if thin:
                    last[j % thin] = acc
                o = acc * inv
                res = o if res is None else res + o
                a_s[asl, r0:r0 + R, j * 128:(j + 1) * 128] = o.astype(BF16)
            if ret:
                return res
        return [functools.partial(job, r) for r in range(ra, rb)]

    def wo_mm(t, xs, toks, r0=0, nr=T, ln=False, asl=0, tok=None):
        att = jnp.dot(a_s[asl, r0:r0 + nr, :], gate_rows(wo_p[...], tok), preferred_element_type=F32)
        tok_of(att, toks, range(NC))
        x1 = x_v[rows(t, r0, nr), :].astype(F32) + mod(2) * att
        x1_s[xs, r0:r0 + nr, :] = x1
        if ln:
            h2_s[r0:r0 + nr, :] = (_ln(x1) * (1.0 + mod(4)) + mod(3)).astype(BF16)

    def out_copy(t):
        return pltpu.make_async_copy(o_v.at[rows(t)], o_hbm.at[rows(t)], sem_out.at[0])

    def out_copy_col(t, j, r0=0, nr=T):
        cs = pl.ds(j * 128, 128)
        return pltpu.make_async_copy(o_v.at[rows(t, r0, nr), cs], o_hbm.at[rows(t, r0, nr), cs], sem_out.at[0])

    class FFN:
        def __init__(self):
            self.us = []
            self.y = None

        def w1(self, c, toks, split=False):
            if split:
                u = jnp.concatenate([
                    jnp.dot(h2_s[hh * (T // 2):(hh + 1) * (T // 2), :], w1_v[c], preferred_element_type=F32)
                    for hh in range(2)], axis=0)
            else:
                u = jnp.dot(h2_s[...], w1_v[c], preferred_element_type=F32)
            tok_of(u, toks, range(FC // 128))
            self.us.append(_silu(u).astype(BF16))

        def w2(self, c, toks):
            p = jnp.dot(self.us[c], w2_v[c], preferred_element_type=F32)
            tok_of(p, toks, (0, 2))
            self.y = p if self.y is None else self.y + p

        def run(self, seq, toks):
            for kind, c in seq:
                (self.w1 if kind == 1 else self.w2)(c, toks)

        def fin(self, t, xs):
            o_v[rows(t), :] = (x1_s[xs] + mod(5) * self.y).astype(BF16)

        def fin_cols(self, t, xs):
            uu = jnp.concatenate(self.us[nch - 2:], axis=1)
            for j in range(NC):
                cs = slice(j * 128, (j + 1) * 128)
                wj = jnp.concatenate([w2_v[nch - 2, :, cs], w2_v[nch - 1, :, cs]], axis=0)
                y = self.y[:, cs] + jnp.dot(uu, wj, preferred_element_type=F32)
                o = (x1_s[xs, :, cs] + mod(5, j * 128, (j + 1) * 128) * y).astype(BF16)
                for r0, nr in ((0, T - LS), (T - LS, LS)) if (LS and j == NC - 1) else ((0, T),):
                    o_v[rows(t, r0, nr), cs] = o[r0:r0 + nr]
                    out_copy_col(t, j, r0, nr).start()

    SEQ = [(1, 0)]
    for c in range(nch):
        if c + 1 < nch:
            SEQ.append((1, c + 1))
        SEQ.append((2, c))

    def body(t, carry):
        sl = (t + 1) & 1
        x_late(t + 3).wait()
        f = FFN()
        toks = []
        f.run(SEQ, toks)
        _spread(_merge(attn_jobs(sl, 0, NR, thin=TH2), ln1_jobs(t + 3, 0, True)), toks[:len(toks) - TA])
        f.fin(t, 0)
        wo_mm(t + 1, 0, [], ln=True)
        for a in range(3):
            qkv_part(a, 0, sl, 1 - sl, [])
        out_copy(t).start()
        return carry

    def fold(h):
        parts = [h[r:r + 8, c:c + 128] for r in range(0, h.shape[0], 8) for c in range(0, h.shape[1], 128)]
        return tsum(parts)

    def ln0_jobs(t, hs, k1):
        def job(r, tok):
            rs = slice(r * LR, (r + 1) * LR)
            y = _ln(_gate(x_v[rows(t, r * LR, LR), :], tok).astype(F32))
            x1_s[hs, rs, k1:] = y[:, k1:]
            h = y[:, :k1] * (1.0 + mod(1, 0, k1)) + mod(0, 0, k1)
            h1_s[hs, rs, :k1] = h.astype(BF16)
            return h[0:8, 0:128] + h[8:16, 0:128] + y[0:8, 256:384] + y[8:16, 384:512]
        return [functools.partial(job, r) for r in range(NL)]

    def mod_jobs(hs, kr):
        nr = LR * KH // (kr[1] - kr[0])

        def job(r, tok):
            rs = slice(r * nr, (r + 1) * nr)
            h = _gate(x1_s[hs, rs, kr[0]:kr[1]], tok) * (1.0 + mod(1, *kr)) + mod(0, *kr)
            h1_s[hs, rs, kr[0]:kr[1]] = h.astype(BF16)
            return fold(h)
        return [functools.partial(job, r) for r in range(T // nr)]

    def calc_piece(kr, nch):
        return tsum(calc_mod(kr, (D + kr[0], D + kr[1]), nch=nch))

    K0, K1, K2 = KP
    K01 = (0, K1[1])
    k_s[2, :, 0:HALO, :] = jnp.zeros((NC, HALO, 128), F32)
    v_s[2, :, 0:HALO, :] = jnp.zeros((NC, HALO, 128), F32)
    wait('c', 'x0')
    add('m1', *mcols(2 * D, 3 * D), 0)
    pairs(0, P0, 0)
    make_sct()
    x1_s[0] = _ln(x_v[rows(0), :].astype(F32))
    wait('sa0', 'ca0')
    add('gb', *mcols(5 * D, D), 1)
    pairs(P0, nch, 1)
    calc_piece(K0, 2)
    _par(mod_jobs(0, K0), [])
    wait('W0')
    x_late(4).start()
    perm_w(K0)
    for a in range(HB):
        qkv_part(a, 0, 2, None, [], K0)
    wait('x12')
    x_late(5).start()
    for a in range(HB, 3):
        qkv_part(a, 0, 2, None, [], K0)
    _par(ln0_jobs(1, 1, K0[1]), [])
    tk = []
    for a in range(3):
        qkv_part(a, 1, 3, None, tk, K0)
    _par(ln0_jobs(2, 2, K0[1]), tk[:6])
    for a in range(HB4):
        qkv_part(a, 2, 0, None, [], K0)
    wait('W1', 'sa1', 'ca1', 'x3')
    x_late(6).start()
    tm = calc_piece(K1, 2)
    for a in range(HB4, 3):
        qkv_part(a, 2, 0, None, [], K0, tm if (a == 2 and HB4 < 2) else None)
    perm_w(K1)
    td = _spread(mod_jobs(0, K1), [])
    tk = []
    qkv_part(0, 0, 2, None, tk, K1, td)
    td = _spread(mod_jobs(1, K1), [td])
    qkv_part(1, 0, 2, None, tk, K1, td)
    td = _spread(mod_jobs(2, K1), [td])
    qkv_part(2, 0, 2, None, tk, K1, td)
    for a in range(3):
        qkv_part(a, 1, 3, None, tk, K1)
    _par(ln0_jobs(3, 3, K1[1]), tk[4:])
    for a in range(3):
        qkv_part(a, 2, 0, None, [], K1)
    qkv_part(2, 3, 1, None, [], K01)
    if QB:
        qkv_part(0, 3, 1, None, [], K01, j1=QB)
    wait('W2', 'sa2', 'ca2', 'wo')
    x_late(7).start()
    tm = calc_piece(K2, CH)
    if QB < NC:
        qkv_part(0, 3, 1, None, [], K01, j0=QB)
    qkv_part(1, 3, 1, None, [], K01, tm if QB == 0 else None)
    perm_w(K2)
    td = _spread(mod_jobs(0, K2), [])
    tk = []
    qkv_part(0, 0, 2, None, tk, K2, td)
    td = _spread(mod_jobs(1, K2), [td])
    qkv_part(1, 0, 2, None, tk, K2, td)
    td = _spread(mod_jobs(2, K2), [td])
    qkv_part(2, 0, 2, None, tk, K2, td)
    td = _spread(mod_jobs(3, K2), [td])
    dots = [(a, 1, 3, 2) for a in range(3)] + [(a, 2, 0, 3) for a in range(3)] + [(a, 3, 1, 0) for a in range(2)]
    jobs = attn_jobs(2, 0, NR, first=True, thin=TH0, ret=True)
    L = [None] + tk[AV:]
    nL = len(L) + 8 * len(dots) - TB
    pj = perm_wo_jobs()
    off = PW0 - AV + 1
    done = []
    k = kp = 0
    for i in range(len(dots) + 1):
        res = []
        while k < NR and k * nL // NR < len(L):
            res.append(jobs[k](L[k * nL // NR]))
            k += 1
        while kp < len(pj) and off + kp * (PW1 - PW0) // len(pj) < len(L):
            q = off + kp * (PW1 - PW0) // len(pj)
            r = pj[kp](L[q] if q > 0 else tk[q + AV - 1])
            if PD:
                res.append(r)
            kp += 1
        done.append(tsum(res) if res else None)
        if i < len(dots):
            g = td if i == 0 else (done[i - DL] if i >= DL else None)
            qkv_part(*dots[i], L, K2, g)
    wait('m1', *[f'w{k}_{c}' for c in range(P0) for k in (1, 2)])
    t1 = calc_mod((2 * D, 3 * D), nch=CH1)
    t2 = calc_mod((4 * D, 5 * D), nch=CH1, last=t1)
    t3 = calc_mod((3 * D, 4 * D), nch=CH1, last=t2)
    gs = [None, tsum(t1), tsum(t2), tsum(t3)]
    wo_mm(0, 1, [], 0, T // 2, ln=True)
    wo_mm(0, 1, [], T // 2, T // 2, ln=True, tok=gs[G1])
    qkv_part(2, 3, 1, 0, [], K2, tok=gs[G2])
    f = FFN()
    toks = []
    seq0 = [s for s in SEQ if s[1] < P0]
    seq1 = [s for s in SEQ if s not in seq0]
    f.run(seq0, toks)
    _spread(attn_jobs(3, A0, A1, asl=1, thin=TH1), toks[:-3])
    wait('gb', *[f'w{k}_{c}' for c in range(P0, nch) for k in (1, 2)])
    tg = tsum(calc_mod((5 * D, 6 * D), nch=1))
    toks = []
    f.run(seq1[:-2], toks)
    _spread(attn_jobs(3, A1, NR, asl=1, thin=TH1), [None] + toks[:-4])
    wo_mm(1, 0, [], ln=True, asl=1, tok=tg)
    f.run(seq1[-2:], [])
    f.fin(0, 1)
    out_copy(0).start()
    lax.fori_loop(1, n - 3, body, 0)
    for t in (n - 3, n - 2):
        xs = (t - n + 3) & 1
        f = FFN()
        toks = []
        f.run(SEQ[:3], toks)
        if t == n - 2:
            out_copy(t - 1).start()
        f.run(SEQ[3:-2], toks)
        _spread(attn_jobs((t + 1) & 1, 0, NR, thin=TH2), toks[:-6])
        wo_mm(t + 1, 1 - xs, [], ln=True)
        f.run(SEQ[-2:], [])
        f.fin(t, xs)
    f = FFN()
    f.run(SEQ[:3], [])
    out_copy(n - 2).start()
    f.run(SEQ[3:-2], [])
    f.fin_cols(n - 1, 0)


A0 = 0
A1 = 14
P0 = 3
HB = 1
KP = ((0, 128), (128, 256), (256, 512))
TB = 10
CH = 2
LS = 128
HB4 = 1
QB = 2
PD = 0
DL = 1
AV = 16
SS = 33
PW0 = 8
PW1 = 80
CH1 = 2
G1 = 1
G2 = 3
TH0 = 2
TH1 = 0
TH2 = 0


@jax.jit
def pallas_adaLN_cond__sliding_local_dilated__dense_activation_silu__prompt_kernel(
    A_x, A_wqkv, A_wo, B_x, B_w1, B_w2, c, w_mod,
):
    B, S, _ = A_x.shape
    Fd = B_w1.shape[1]
    n = S // T
    nch = Fd // FC
    assert n == 8
    x2 = A_x.reshape(S, D)
    anyspec = pl.BlockSpec(memory_space=pl.ANY)
    out = pl.pallas_call(
        functools.partial(_kernel, n=n, nch=nch),
        in_specs=[anyspec] * 7,
        out_specs=anyspec,
        out_shape=jax.ShapeDtypeStruct((S, D), A_x.dtype),
        scratch_shapes=[
            pltpu.VMEM((S, D), BF16),
            pltpu.VMEM((S, D), BF16),
            pltpu.VMEM((D, 3 * D), BF16),
            pltpu.VMEM((D, D), BF16),
            pltpu.VMEM((nch, D, FC), BF16),
            pltpu.VMEM((nch, FC, D), BF16),
            pltpu.VMEM((1, D), BF16),
            pltpu.VMEM((D, 6 * D), BF16),
            pltpu.VMEM((D // 2, 3 * D), U32),
            pltpu.VMEM((D, D), BF16),
            pltpu.VMEM((NC, DH * 40, 128), F32),
            pltpu.VMEM((1, 6 * D), F32),
            pltpu.VMEM((D, 128), F32),
            pltpu.VMEM((SLOTS, NC, T, 128), F32),
            pltpu.VMEM((SLOTS, NC, T + HALO, 128), F32),
            pltpu.VMEM((SLOTS, NC, T + HALO, 128), F32),
            pltpu.VMEM((2, T, D), BF16),
            pltpu.VMEM((4, T, D), BF16),
            pltpu.VMEM((T, D), BF16),
            pltpu.VMEM((4, T, D), F32),
            pltpu.SemaphoreType.DMA((1,)),
        ],
        compiler_params=pltpu.CompilerParams(vmem_limit_bytes=100 * 1024 * 1024),
    )(x2, A_wqkv, A_wo, B_w1, B_w2, c, w_mod)
    return out.reshape(B, S, D)
```
